```python
import jax
import jax.numpy as jnp

def _softmax(x, axis=-1):
    return jax.nn.softmax(x, axis=axis)
def _gelu(x):
    return jax.nn.gelu(x, approximate=True)
def _silu(x):
    return jax.nn.silu(x)
def _sigmoid(x):
    return jax.nn.sigmoid(x)
def _layernorm(x, axis=-1, eps=1e-5):
    m = jnp.mean(x, axis=axis, keepdims=True)
    v = jnp.var(x, axis=axis, keepdims=True)
    return (x - m) / jnp.sqrt(v + eps)
def _scatter_add(tgt, idx, src, axis=0):
    return tgt.at[idx].add(src)
def _segment_sum(src, seg, n):
    return jax.ops.segment_sum(src, seg, n)
class _Rng:
    def __init__(self, key):
        self._k = key
    def _next(self):
        self._k, sub = jax.random.split(self._k)
        return sub
    def normal(self, shape):
        return jax.random.normal(self._next(), shape, dtype=jnp.bfloat16)
    def randint(self, lo, hi, shape):
        return jax.random.randint(self._next(), shape, lo, hi, dtype=jnp.int32)
    def uniform(self, shape, lo=0.0, hi=1.0):
        return jax.random.uniform(self._next(), shape, jnp.bfloat16, lo, hi)
    def permutation(self, n):
        return jax.random.permutation(self._next(), n)


kernel_name = 'parallel_sum__sliding_block_cached__moe_arch_mod__decode'

def setup_inputs():
    _rng = _Rng(jax.random.key(int.from_bytes(__import__("os").urandom(4), "little")))
    _w = (lambda a: (lambda t: t.astype(jnp.bfloat16) if jnp.issubdtype(t.dtype, jnp.floating) else t)(jnp.asarray(a)))
    def _A_setup():
        B, Sq, D = 1, 1, 512
        Hq, Hkv, Sk, Dh = 32, 8, 65536, 128
        assert Hq % Hkv == 0, (Hq, Hkv)
        return {
            "x": _w((lambda *s: _rng.normal(s) * 0.05)(B, Sq, D)),
            "k_cache": _w((lambda *s: _rng.normal(s) * 0.05)(B, Hkv, Sk, Dh)),
            "v_cache": _w((lambda *s: _rng.normal(s) * 0.05)(B, Hkv, Sk, Dh)),
            "wq": _w((lambda *s: _rng.normal(s) * 0.05)(D, Hq * Dh) * (D ** -0.5)),
            "wo": _w((lambda *s: _rng.normal(s) * 0.05)(Hq * Dh, D) * ((Hq * Dh) ** -0.5)),
        }
    _A_in = _A_setup()

    def _B_setup():
        B, S, D, F, C = 1, 1, 512, 1792, 1
        return {
            "x": _w((lambda *s: _rng.normal(s) * 0.05)(B, S, D)),
            "w_r": _w((lambda *s: _rng.normal(s) * 0.05)(D)),
            "w_gate": _w((lambda *s: _rng.normal(s) * 0.05)(D, F)),
            "w_up": _w((lambda *s: _rng.normal(s) * 0.05)(D, F)),
            "w_down": _w((lambda *s: _rng.normal(s) * 0.05)(F, D)),
        }
    _B_in = _B_setup()

    return {
        "A_x": _A_in["x"],
        "A_k_cache": _A_in["k_cache"],
        "A_v_cache": _A_in["v_cache"],
        "A_wq": _A_in["wq"],
        "A_wo": _A_in["wo"],
        "B_x": _B_in["x"],
        "B_w_r": _B_in["w_r"],
        "B_w_gate": _B_in["w_gate"],
        "B_w_up": _B_in["w_up"],
        "B_w_down": _B_in["w_down"],
    }

def reference(A_x, A_k_cache, A_v_cache, A_wq, A_wo, B_x, B_w_r, B_w_gate, B_w_up, B_w_down):
    def _A_ref(x, k_cache, v_cache, wq, wo):
        B, Sq, D = x.shape
        Hq, Dh = 32, 128
        Hkv, Sk = k_cache.shape[1], k_cache.shape[2]
        W = min(4096, max(256, Sk // 4))
        rep = Hq // Hkv
        q = (lambda x, *d: x.transpose(*d))((x @ wq).reshape(B, Sq, Hq, Dh), 0, 2, 1, 3)
        k = jnp.repeat(k_cache[:, :, Sk - W:, :], rep, axis=1)
        v = jnp.repeat(v_cache[:, :, Sk - W:, :], rep, axis=1)
        scores = jnp.einsum("bhqd,bhkd->bhqk", q, k) * (Dh ** -0.5)
        p = _softmax(scores, axis=-1)
        o = jnp.einsum("bhqk,bhkd->bhqd", p, v)
        return (lambda x, *d: x.transpose(*d))(o, 0, 2, 1, 3).reshape(B, Sq, Hq * Dh) @ wo

    def _B_ref(x, w_r, w_gate, w_up, w_down):
        B, S, D = x.shape
        C = 1
        r = x @ w_r
        idx = jnp.argsort(-r, axis=-1)[:, :C]
        idx_e = jnp.repeat(idx.reshape(B, C, 1), D, axis=2)
        x_sel = jnp.take_along_axis(x, idx_e, axis=1)
        g = _silu(x_sel @ w_gate)
        u = x_sel @ w_up
        y = (g * u) @ w_down
        r_sel = _sigmoid(jnp.take_along_axis(r, idx, axis=1))
        y = y * r_sel.reshape(B, C, 1)
        b_off = (jnp.arange(B) * S).reshape(B, 1)
        flat_idx = (idx + b_off).reshape(B * C)
        zero = (x * 0.0).reshape(B * S, D)
        upd = _scatter_add(zero, flat_idx, y.reshape(B * C, D), axis=0)
        return x + upd.reshape(B, S, D)

    x = A_x
    xn = _layernorm(x, axis=-1)
    return x + _A_ref(xn, A_k_cache, A_v_cache, A_wq, A_wo) + _B_ref(xn, B_w_r, B_w_gate, B_w_up, B_w_down)
```

```python
import jax
import jax.numpy as jnp
from jax import lax
import jax.experimental.pallas as pl
import jax.experimental.pallas.tpu as pltpu

_F32 = jnp.float32
_BF16 = jnp.bfloat16


def _dot(a, b):
    return jnp.dot(a, b, preferred_element_type=_F32)


def _dot_nt(a, b):
    return lax.dot_general(a, b, (((1,), (1,)), ((), ())), preferred_element_type=_F32)


@jax.jit
def pallas_parallel_sum__sliding_block_cached__moe_arch_mod__decode_kernel(
    A_x: jax.Array,
    A_k_cache: jax.Array,
    A_v_cache: jax.Array,
    A_wq: jax.Array,
    A_wo: jax.Array,
    B_x: jax.Array,
    B_w_r: jax.Array,
    B_w_gate: jax.Array,
    B_w_up: jax.Array,
    B_w_down: jax.Array,
):
    del B_x
    B, Sq, D = A_x.shape
    Hq, Dh = 32, 128
    Hkv, Sk = A_k_cache.shape[1], A_k_cache.shape[2]
    W = min(4096, max(256, Sk // 4))
    rep = Hq // Hkv
    F = B_w_gate.shape[1]
    assert B == 1 and Sq == 1 and rep <= 8
    R = 8
    scale = Dh ** -0.5
    G = rep * Dh

    wo_chunks = [(0, 2048), (2048, 1024), (3072, 512), (3584, 256), (3840, 128), (3968, 128)]

    def kernel(x_hbm, wr_hbm, k_hbm, v_hbm, wq_hbm, wo_hbm, wg_hbm, wu_hbm, wd_hbm,
               o_ref,
               xb, wrb, kb, vb, wqb, wob, wgb, wub, wdb, sems):
        copies = {}

        def add(name, src, dst):
            copies[name] = pltpu.make_async_copy(src, dst, sems.at[len(copies)])

        add("x", x_hbm, xb)
        add("wr", wr_hbm, wrb)
        add("wq", wq_hbm, wqb)
        for h in range(Hkv):
            add(("k", h), k_hbm.at[0, h, pl.ds(Sk - W, W)], kb.at[h])
            add(("v", h), v_hbm.at[0, h, pl.ds(Sk - W, W)], vb.at[h])
        add("wg", wg_hbm, wgb)
        add("wu", wu_hbm, wub)
        add("wd", wd_hbm, wdb)
        for (r0, n) in wo_chunks:
            add(("wo", r0), wo_hbm.at[pl.ds(r0, n)], wob.at[pl.ds(r0, n)])
        for c in copies.values():
            c.start()

        copies["x"].wait()
        copies["wr"].wait()
        x = xb[...].astype(_F32)
        m = jnp.mean(x, axis=-1, keepdims=True)
        xc = x - m
        var = jnp.mean(xc * xc, axis=-1, keepdims=True)
        xn = xc / jnp.sqrt(var + 1e-5)
        xn_bf = xn.astype(_BF16)
        xn = xn_bf.astype(_F32)
        xn8 = jnp.broadcast_to(xn, (R, D)).astype(_BF16)
        wr = wrb[...].astype(_F32)
        racc = xn[:, 0:128] * wr[0:1, :]
        for j in range(1, D // 128):
            racc = racc + xn[:, j * 128:(j + 1) * 128] * wr[j:j + 1, :]
        r = jnp.sum(racc, axis=-1, keepdims=True)
        r_sel = jax.nn.sigmoid(r)

        row = lax.broadcasted_iota(jnp.int32, (R, Dh), 0)

        copies["wq"].wait()
        q8 = _dot(xn8, wqb[...])

        lhs_o = []
        for h in range(Hkv):
            qh = q8[:, h * G:h * G + Dh]
            for j in range(1, rep):
                qh = jnp.where(row == j, q8[:, h * G + j * Dh:h * G + (j + 1) * Dh], qh)
            qh = qh.astype(_BF16)
            copies[("k", h)].wait()
            s = _dot_nt(qh, kb[h]) * scale
            mx = jnp.max(s, axis=-1, keepdims=True)
            p = jnp.exp(s - mx)
            l = jnp.sum(p, axis=-1, keepdims=True)
            copies[("v", h)].wait()
            oh = _dot(p.astype(_BF16), vb[h]) / l
            for j in range(rep):
                lhs_o.append(jnp.where(row == j, oh, 0.0).astype(_BF16))
        lo = jnp.concatenate(lhs_o, axis=1)

        copies["wg"].wait()
        g = _dot(xn8, wgb[...])
        copies["wu"].wait()
        u = _dot(xn8, wub[...])
        hh = (g * jax.nn.sigmoid(g) * u).astype(_BF16)
        copies["wd"].wait()
        y = _dot(hh, wdb[...])[0:1, :] * r_sel
        base = x + xn + y

        acc = None
        for (r0, n) in wo_chunks:
            copies[("wo", r0)].wait()
            part = _dot(lo[:, r0:r0 + n], wob[pl.ds(r0, n), :])
            acc = part if acc is None else acc + part
        attn = jnp.sum(acc, axis=0, keepdims=True)
        o_ref[...] = (base + attn).astype(o_ref.dtype)

    n_copies = 3 + 2 * Hkv + 3 + len(wo_chunks)
    any_spec = pl.BlockSpec(memory_space=pl.ANY)
    out = pl.pallas_call(
        kernel,
        out_shape=jax.ShapeDtypeStruct((1, D), A_x.dtype),
        in_specs=[any_spec] * 9,
        out_specs=pl.BlockSpec(memory_space=pltpu.VMEM),
        scratch_shapes=[
            pltpu.VMEM((1, D), _BF16),
            pltpu.VMEM((D // 128, 128), _BF16),
            pltpu.VMEM((Hkv, W, Dh), _BF16),
            pltpu.VMEM((Hkv, W, Dh), _BF16),
            pltpu.VMEM((D, Hq * Dh), _BF16),
            pltpu.VMEM((Hq * Dh, D), _BF16),
            pltpu.VMEM((D, F), _BF16),
            pltpu.VMEM((D, F), _BF16),
            pltpu.VMEM((F, D), _BF16),
            pltpu.SemaphoreType.DMA((n_copies,)),
        ],
        compiler_params=pltpu.CompilerParams(vmem_limit_bytes=64 * 1024 * 1024),
    )(A_x.reshape(1, D), B_w_r.reshape(D // 128, 128), A_k_cache, A_v_cache, A_wq, A_wo,
      B_w_gate, B_w_up, B_w_down)
    return out.reshape(B, Sq, D)
```

```python
import jax
import jax.numpy as jnp
from jax import lax
import jax.experimental.pallas as pl
import jax.experimental.pallas.tpu as pltpu

_F32 = jnp.float32
_BF16 = jnp.bfloat16


def _dot(a, b):
    return jnp.dot(a, b, preferred_element_type=_F32)


def _dot_nt(a, b):
    return lax.dot_general(a, b, (((1,), (1,)), ((), ())), preferred_element_type=_F32)


@jax.jit
def pallas_parallel_sum__sliding_block_cached__moe_arch_mod__decode_kernel(
    A_x: jax.Array,
    A_k_cache: jax.Array,
    A_v_cache: jax.Array,
    A_wq: jax.Array,
    A_wo: jax.Array,
    B_x: jax.Array,
    B_w_r: jax.Array,
    B_w_gate: jax.Array,
    B_w_up: jax.Array,
    B_w_down: jax.Array,
):
    del B_x
    B, Sq, D = A_x.shape
    Hq, Dh = 32, 128
    Hkv, Sk = A_k_cache.shape[1], A_k_cache.shape[2]
    W = min(4096, max(256, Sk // 4))
    rep = Hq // Hkv
    F = B_w_gate.shape[1]
    assert B == 1 and Sq == 1 and rep <= 8
    R = 8
    scale = Dh ** -0.5
    G = rep * Dh

    wo_chunks = [(0, 2048), (2048, 1024), (3072, 512), (3584, 256), (3840, 128), (3968, 128)]

    def kernel(*refs):
        pl.run_scoped(lambda sems: body(*refs, sems),
                      pltpu.SemaphoreType.DMA((n_copies,)))

    def body(x_hbm, wr_hbm, k_hbm, v_hbm, wq_hbm, wo_hbm, wg_hbm, wu_hbm, wd_hbm,
             o_ref,
             xb, wrb, kb, vb, wqb, wob, wgb, wub, wdb, sems):
        copies = {}

        def add(name, src, dst):
            copies[name] = pltpu.make_async_copy(src, dst, sems.at[len(copies)])

        add("x", x_hbm, xb)
        add("wr", wr_hbm, wrb)
        add("wq", wq_hbm, wqb)
        for h in range(Hkv):
            add(("k", h), k_hbm.at[0, h, pl.ds(Sk - W, W)], kb.at[h])
            add(("v", h), v_hbm.at[0, h, pl.ds(Sk - W, W)], vb.at[h])
        add("wg", wg_hbm, wgb)
        add("wu", wu_hbm, wub)
        add("wd", wd_hbm, wdb)
        for (r0, n) in wo_chunks:
            add(("wo", r0), wo_hbm.at[pl.ds(r0, n)], wob.at[pl.ds(r0, n)])
        for c in copies.values():
            c.start()

        copies["x"].wait()
        copies["wr"].wait()
        x = xb[...].astype(_F32)
        m = jnp.mean(x, axis=-1, keepdims=True)
        xc = x - m
        var = jnp.mean(xc * xc, axis=-1, keepdims=True)
        xn = xc / jnp.sqrt(var + 1e-5)
        xn_bf = xn.astype(_BF16)
        xn = xn_bf.astype(_F32)
        xn8 = jnp.broadcast_to(xn, (R, D)).astype(_BF16)
        wr = wrb[...].astype(_F32)
        racc = xn[:, 0:128] * wr[0:1, :]
        for j in range(1, D // 128):
            racc = racc + xn[:, j * 128:(j + 1) * 128] * wr[j:j + 1, :]
        r = jnp.sum(racc, axis=-1, keepdims=True)
        r_sel = jax.nn.sigmoid(r)

        row = lax.broadcasted_iota(jnp.int32, (R, Dh), 0)

        copies["wq"].wait()
        q8 = _dot(xn8, wqb[...])

        lhs_o = []
        for h in range(Hkv):
            qh = q8[:, h * G:h * G + Dh]
            for j in range(1, rep):
                qh = jnp.where(row == j, q8[:, h * G + j * Dh:h * G + (j + 1) * Dh], qh)
            qh = qh.astype(_BF16)
            copies[("k", h)].wait()
            s = _dot_nt(qh, kb[h]) * scale
            mx = jnp.max(s, axis=-1, keepdims=True)
            p = jnp.exp(s - mx)
            l = jnp.sum(p, axis=-1, keepdims=True)
            copies[("v", h)].wait()
            oh = _dot(p.astype(_BF16), vb[h]) / l
            for j in range(rep):
                lhs_o.append(jnp.where(row == j, oh, 0.0).astype(_BF16))
        lo = jnp.concatenate(lhs_o, axis=1)

        copies["wg"].wait()
        g = _dot(xn8, wgb[...])
        copies["wu"].wait()
        u = _dot(xn8, wub[...])
        hh = (g * jax.nn.sigmoid(g) * u).astype(_BF16)
        copies["wd"].wait()
        y = _dot(hh, wdb[...])[0:1, :] * r_sel
        base = x + xn + y

        acc = None
        for (r0, n) in wo_chunks:
            copies[("wo", r0)].wait()
            part = _dot(lo[:, r0:r0 + n], wob[pl.ds(r0, n), :])
            acc = part if acc is None else acc + part
        attn = jnp.sum(acc, axis=0, keepdims=True)
        o_ref[...] = (base + attn).astype(o_ref.dtype)

    n_copies = 3 + 2 * Hkv + 3 + len(wo_chunks)
    any_spec = pl.BlockSpec(memory_space=pl.ANY)
    out = pl.pallas_call(
        kernel,
        out_shape=jax.ShapeDtypeStruct((1, D), A_x.dtype),
        in_specs=[any_spec] * 9,
        out_specs=pl.BlockSpec(memory_space=pltpu.VMEM),
        scratch_shapes=[
            pltpu.VMEM((1, D), _BF16),
            pltpu.VMEM((D // 128, 128), _BF16),
            pltpu.VMEM((Hkv, W, Dh), _BF16),
            pltpu.VMEM((Hkv, W, Dh), _BF16),
            pltpu.VMEM((D, Hq * Dh), _BF16),
            pltpu.VMEM((Hq * Dh, D), _BF16),
            pltpu.VMEM((D, F), _BF16),
            pltpu.VMEM((D, F), _BF16),
            pltpu.VMEM((F, D), _BF16),
        ],
        compiler_params=pltpu.CompilerParams(vmem_limit_bytes=64 * 1024 * 1024),
    )(A_x.reshape(1, D), B_w_r.reshape(D // 128, 128), A_k_cache, A_v_cache, A_wq, A_wo,
      B_w_gate, B_w_up, B_w_down)
    return out.reshape(B, Sq, D)
```

```python
import jax
import jax.numpy as jnp
from jax import lax
import jax.experimental.pallas as pl
import jax.experimental.pallas.tpu as pltpu

_F32 = jnp.float32
_BF16 = jnp.bfloat16
_LANES = 128
_SUB = 8


def _dot(a, b):
    return jnp.dot(a, b, preferred_element_type=_F32)


def _dot_nt(a, b):
    return lax.dot_general(a, b, (((1,), (1,)), ((), ())), preferred_element_type=_F32)


def _tree_sum(xs):
    xs = list(xs)
    while len(xs) > 1:
        nxt = [xs[i] + xs[i + 1] for i in range(0, len(xs) - 1, 2)]
        if len(xs) % 2:
            nxt.append(xs[-1])
        xs = nxt
    return xs[0]


@jax.jit
def pallas_parallel_sum__sliding_block_cached__moe_arch_mod__decode_kernel(
    A_x: jax.Array,
    A_k_cache: jax.Array,
    A_v_cache: jax.Array,
    A_wq: jax.Array,
    A_wo: jax.Array,
    B_x: jax.Array,
    B_w_r: jax.Array,
    B_w_gate: jax.Array,
    B_w_up: jax.Array,
    B_w_down: jax.Array,
):
    del B_x
    B, Sq, D = A_x.shape
    Hq, Dh = 32, 128
    Hkv, Sk = A_k_cache.shape[1], A_k_cache.shape[2]
    W = min(4096, max(256, Sk // 4))
    rep = Hq // Hkv
    F = B_w_gate.shape[1]
    assert B == 1 and Sq == 1 and rep <= _SUB and Dh == _LANES and D % _LANES == 0
    R = _SUB
    scale = Dh ** -0.5
    G = rep * Dh
    NC = D // _LANES

    wo_mxu = [(0, 2048), (2048, 1024), (3072, 512), (3584, 256), (3840, 128)]
    wo_vpu = [(3968, 64), (4032, 32), (4064, 16), (4080, 16)]
    vpu_base = wo_vpu[0][0]
    assert vpu_base == (Hq - 1) * Dh
    n_copies = 3 + 2 * Hkv + 3 + len(wo_mxu) + len(wo_vpu)

    def kernel(*refs):
        pl.run_scoped(lambda sems: body(*refs, sems),
                      pltpu.SemaphoreType.DMA((n_copies,)))

    def body(x_hbm, wr_hbm, k_hbm, v_hbm, wq_hbm, wo_hbm, wg_hbm, wu_hbm, wd_hbm,
             o_ref,
             xb, wrb, kb, vb, wqb, wob, wgb, wub, wdb, coef_ref, sems):
        copies = {}

        def add(name, src, dst):
            copies[name] = pltpu.make_async_copy(src, dst, sems.at[len(copies)])

        add("x", x_hbm, xb)
        add("wr", wr_hbm, wrb)
        add("wq", wq_hbm, wqb)
        for h in range(Hkv):
            add(("k", h), k_hbm.at[0, h, pl.ds(Sk - W, W)], kb.at[h])
            add(("v", h), v_hbm.at[0, h, pl.ds(Sk - W, W)], vb.at[h])
        add("wg", wg_hbm, wgb)
        add("wu", wu_hbm, wub)
        add("wd", wd_hbm, wdb)
        for (r0, n) in wo_mxu + wo_vpu:
            add(("wo", r0), wo_hbm.at[pl.ds(r0, n)], wob.at[pl.ds(r0, n)])
        assert len(copies) == n_copies
        for c in copies.values():
            c.start()

        copies["x"].wait()
        copies["wr"].wait()
        x = xb[...].astype(_F32)
        m = jnp.mean(x, axis=-1, keepdims=True)
        xc = x - m
        var = jnp.mean(xc * xc, axis=-1, keepdims=True)
        xn = xc / jnp.sqrt(var + 1e-5)
        xn = xn.astype(_BF16).astype(_F32)
        xn8 = jnp.broadcast_to(xn, (R, D)).astype(_BF16)
        wr = wrb[...].astype(_F32)
        racc = xn[:, 0:_LANES] * wr[0:1, :]
        for j in range(1, NC):
            racc = racc + xn[:, j * _LANES:(j + 1) * _LANES] * wr[j:j + 1, :]
        r = jnp.sum(racc, axis=-1, keepdims=True)
        r_sel = jax.nn.sigmoid(r)

        row = lax.broadcasted_iota(jnp.int32, (R, Dh), 0)

        copies["wq"].wait()
        q8 = _dot(xn8, wqb[...])

        lhs_o = []
        for h in range(Hkv):
            qh = q8[:, h * G:h * G + Dh]
            for j in range(1, rep):
                qh = jnp.where(row == j, q8[:, h * G + j * Dh:h * G + (j + 1) * Dh], qh)
            qh = qh.astype(_BF16)
            copies[("k", h)].wait()
            s = _dot_nt(qh, kb[h]) * scale
            mx = jnp.max(s, axis=-1, keepdims=True)
            p = jnp.exp(s - mx)
            l = jnp.sum(p, axis=-1, keepdims=True)
            copies[("v", h)].wait()
            oh = _dot(p.astype(_BF16), vb[h]) / l
            for j in range(rep):
                if h * rep + j < Hq - 1:
                    lhs_o.append(jnp.where(row == j, oh, 0.0).astype(_BF16))
                else:
                    o_last = oh[j:j + 1, :].astype(_BF16).astype(_F32)
                    coef_ref[...] = jnp.broadcast_to(o_last, (Dh, Dh)).T
        lo = jnp.concatenate(lhs_o, axis=1)

        copies["wg"].wait()
        g = _dot(xn8, wgb[...])
        copies["wu"].wait()
        u = _dot(xn8, wub[...])
        hh = (g * jax.nn.sigmoid(g) * u).astype(_BF16)
        copies["wd"].wait()
        y = _dot(hh, wdb[...]) * r_sel
        row_d = lax.broadcasted_iota(jnp.int32, (R, D), 0)
        acc = jnp.where(row_d == 0, (x + xn) + y, 0.0)

        for (r0, n) in wo_mxu:
            copies[("wo", r0)].wait()
            acc = acc + _dot(lo[:, r0:r0 + n], wob[pl.ds(r0, n), :])
        accs = [acc[:, c * _LANES:(c + 1) * _LANES] for c in range(NC)]
        for (r0, n) in wo_vpu:
            cf = [coef_ref[pl.ds(r0 - vpu_base + i, _SUB), :] for i in range(0, n, _SUB)]
            copies[("wo", r0)].wait()
            w = wob[pl.ds(r0, n), :].astype(_F32)
            for c in range(NC):
                prods = [w[i * _SUB:(i + 1) * _SUB, c * _LANES:(c + 1) * _LANES] * cf[i]
                         for i in range(n // _SUB)]
                accs[c] = accs[c] + _tree_sum(prods)
        res = jnp.sum(jnp.concatenate(accs, axis=1), axis=0, keepdims=True)
        o_ref[...] = res.astype(o_ref.dtype)

    any_spec = pl.BlockSpec(memory_space=pl.ANY)
    out = pl.pallas_call(
        kernel,
        out_shape=jax.ShapeDtypeStruct((1, D), A_x.dtype),
        in_specs=[any_spec] * 9,
        out_specs=pl.BlockSpec(memory_space=pltpu.VMEM),
        scratch_shapes=[
            pltpu.VMEM((1, D), _BF16),
            pltpu.VMEM((NC, _LANES), _BF16),
            pltpu.VMEM((Hkv, W, Dh), _BF16),
            pltpu.VMEM((Hkv, W, Dh), _BF16),
            pltpu.VMEM((D, Hq * Dh), _BF16),
            pltpu.VMEM((Hq * Dh, D), _BF16),
            pltpu.VMEM((D, F), _BF16),
            pltpu.VMEM((D, F), _BF16),
            pltpu.VMEM((F, D), _BF16),
            pltpu.VMEM((Dh, Dh), _F32),
        ],
        compiler_params=pltpu.CompilerParams(vmem_limit_bytes=64 * 1024 * 1024),
    )(A_x.reshape(1, D), B_w_r.reshape(NC, _LANES), A_k_cache, A_v_cache, A_wq, A_wo,
      B_w_gate, B_w_up, B_w_down)
    return out.reshape(B, Sq, D)
```

```python
import jax
import jax.numpy as jnp
from jax import lax
import jax.experimental.pallas as pl
import jax.experimental.pallas.tpu as pltpu

_F32 = jnp.float32
_BF16 = jnp.bfloat16
_LANES = 128
_SUB = 8


def _dot(a, b):
    return jnp.dot(a, b, preferred_element_type=_F32)


def _dot_nt(a, b):
    return lax.dot_general(a, b, (((1,), (1,)), ((), ())), preferred_element_type=_F32)


def _tree_sum(xs):
    xs = list(xs)
    while len(xs) > 1:
        nxt = [xs[i] + xs[i + 1] for i in range(0, len(xs) - 1, 2)]
        if len(xs) % 2:
            nxt.append(xs[-1])
        xs = nxt
    return xs[0]


@jax.jit
def pallas_parallel_sum__sliding_block_cached__moe_arch_mod__decode_kernel(
    A_x: jax.Array,
    A_k_cache: jax.Array,
    A_v_cache: jax.Array,
    A_wq: jax.Array,
    A_wo: jax.Array,
    B_x: jax.Array,
    B_w_r: jax.Array,
    B_w_gate: jax.Array,
    B_w_up: jax.Array,
    B_w_down: jax.Array,
):
    del B_x
    B, Sq, D = A_x.shape
    Hq, Dh = 32, 128
    Hkv, Sk = A_k_cache.shape[1], A_k_cache.shape[2]
    W = min(4096, max(256, Sk // 4))
    rep = Hq // Hkv
    F = B_w_gate.shape[1]
    assert B == 1 and Sq == 1 and Hkv == 8 and Dh == _LANES and D % _LANES == 0
    R = _SUB
    scale = Dh ** -0.5
    G = rep * Dh
    NC = D // _LANES

    side = [(0, 256, "start", "wq"), (256, 256, "wq", "v3"), (512, 256, "v3", "v7")]
    S = side[-1][0] + side[-1][1]
    wo_mxu = [(S, 2048 - S), (2048, 1024), (3072, 512), (3584, 256), (3840, 128)]
    wo_vpu = [(3968, 64), (4032, 32), (4064, 16), (4080, 16)]
    vpu_base = wo_vpu[0][0]
    assert vpu_base == (Hq - 1) * Dh
    n_copies = 3 + 2 * Hkv + 3 + len(wo_mxu) + len(wo_vpu) + 2 * len(side)

    def kernel(*refs):
        pl.run_scoped(lambda sems: body(*refs, sems),
                      pltpu.SemaphoreType.DMA((n_copies,)))

    def body(x_hbm, wr_hbm, k_hbm, v_hbm, wq_hbm, wo_hbm, wg_hbm, wu_hbm, wd_hbm,
             o_ref,
             xb, wrb, kb, vb, wqb, wob, wgb, wub, wdb, coef_ref, stage, sems):
        copies = {}

        def add(name, src, dst):
            copies[name] = pltpu.make_async_copy(src, dst, sems.at[len(copies)])

        add("wq", wq_hbm, wqb)
        add("x", x_hbm, xb)
        add("wr", wr_hbm, wrb)
        for h in range(Hkv):
            add("k%d" % h, k_hbm.at[0, h, pl.ds(Sk - W, W)], kb.at[h])
            add("v%d" % h, v_hbm.at[0, h, pl.ds(Sk - W, W)], vb.at[h])
        add("wg", wg_hbm, wgb)
        add("wu", wu_hbm, wub)
        add("wd", wd_hbm, wdb)
        for (r0, n) in wo_mxu + wo_vpu:
            add("wo%d" % r0, wo_hbm.at[pl.ds(r0, n)], wob.at[pl.ds(r0, n)])
        main = list(copies)
        for (r0, n, _, _) in side:
            add("h2s%d" % r0, wo_hbm.at[pl.ds(r0, n)], stage.at[pl.ds(r0, n)])
            add("s2v%d" % r0, stage.at[pl.ds(r0, n)], wob.at[pl.ds(r0, n)])
        assert len(copies) == n_copies

        def side_step(event):
            for (r0, _, _, e_s2v) in side:
                if e_s2v == event:
                    copies["h2s%d" % r0].wait()
                    copies["s2v%d" % r0].start()
            for (r0, _, e_h2s, _) in side:
                if e_h2s == event:
                    copies["h2s%d" % r0].start()

        def wait(name):
            copies[name].wait()
            side_step(name)

        copies[main[0]].start()
        side_step("start")
        for name in main[1:]:
            copies[name].start()

        wait("wq")
        wait("x")
        wait("wr")
        x = xb[...].astype(_F32)
        m = jnp.mean(x, axis=-1, keepdims=True)
        xc = x - m
        var = jnp.mean(xc * xc, axis=-1, keepdims=True)
        xn = xc / jnp.sqrt(var + 1e-5)
        xn = xn.astype(_BF16).astype(_F32)
        xn8 = jnp.broadcast_to(xn, (R, D)).astype(_BF16)
        wr = wrb[...].astype(_F32)
        racc = xn[:, 0:_LANES] * wr[0:1, :]
        for j in range(1, NC):
            racc = racc + xn[:, j * _LANES:(j + 1) * _LANES] * wr[j:j + 1, :]
        r = jnp.sum(racc, axis=-1, keepdims=True)
        r_sel = jax.nn.sigmoid(r)

        row = lax.broadcasted_iota(jnp.int32, (R, Dh), 0)

        q8 = _dot(xn8, wqb[...])

        lhs_o = []
        for h in range(Hkv):
            qh = q8[:, h * G:h * G + Dh]
            for j in range(1, rep):
                qh = jnp.where(row == j, q8[:, h * G + j * Dh:h * G + (j + 1) * Dh], qh)
            qh = qh.astype(_BF16)
            wait("k%d" % h)
            s = _dot_nt(qh, kb[h]) * scale
            mx = jnp.max(s, axis=-1, keepdims=True)
            p = jnp.exp(s - mx)
            l = jnp.sum(p, axis=-1, keepdims=True)
            wait("v%d" % h)
            oh = _dot(p.astype(_BF16), vb[h]) / l
            for j in range(rep):
                if h * rep + j < Hq - 1:
                    lhs_o.append(jnp.where(row == j, oh, 0.0).astype(_BF16))
                else:
                    o_last = oh[j:j + 1, :].astype(_BF16).astype(_F32)
                    coef_ref[...] = jnp.broadcast_to(o_last, (Dh, Dh)).T
        lo = jnp.concatenate(lhs_o, axis=1)

        wait("wg")
        g = _dot(xn8, wgb[...])
        wait("wu")
        u = _dot(xn8, wub[...])
        hh = (g * jax.nn.sigmoid(g) * u).astype(_BF16)
        wait("wd")
        y = _dot(hh, wdb[...]) * r_sel
        row_d = lax.broadcasted_iota(jnp.int32, (R, D), 0)
        acc = jnp.where(row_d == 0, (x + xn) + y, 0.0)

        for (r0, _, _, _) in side:
            copies["s2v%d" % r0].wait()
        acc = acc + _dot(lo[:, 0:S], wob[pl.ds(0, S), :])
        for (r0, n) in wo_mxu:
            wait("wo%d" % r0)
            acc = acc + _dot(lo[:, r0:r0 + n], wob[pl.ds(r0, n), :])
        accs = [acc[:, c * _LANES:(c + 1) * _LANES] for c in range(NC)]
        for (r0, n) in wo_vpu:
            cf = [coef_ref[pl.ds(r0 - vpu_base + i, _SUB), :] for i in range(0, n, _SUB)]
            wait("wo%d" % r0)
            w = wob[pl.ds(r0, n), :].astype(_F32)
            for c in range(NC):
                prods = [w[i * _SUB:(i + 1) * _SUB, c * _LANES:(c + 1) * _LANES] * cf[i]
                         for i in range(n // _SUB)]
                accs[c] = accs[c] + _tree_sum(prods)
        res = jnp.sum(jnp.concatenate(accs, axis=1), axis=0, keepdims=True)
        o_ref[...] = res.astype(o_ref.dtype)

    any_spec = pl.BlockSpec(memory_space=pl.ANY)
    out = pl.pallas_call(
        kernel,
        out_shape=jax.ShapeDtypeStruct((1, D), A_x.dtype),
        in_specs=[any_spec] * 9,
        out_specs=pl.BlockSpec(memory_space=pltpu.VMEM),
        scratch_shapes=[
            pltpu.VMEM((1, D), _BF16),
            pltpu.VMEM((NC, _LANES), _BF16),
            pltpu.VMEM((Hkv, W, Dh), _BF16),
            pltpu.VMEM((Hkv, W, Dh), _BF16),
            pltpu.VMEM((D, Hq * Dh), _BF16),
            pltpu.VMEM((Hq * Dh, D), _BF16),
            pltpu.VMEM((D, F), _BF16),
            pltpu.VMEM((D, F), _BF16),
            pltpu.VMEM((F, D), _BF16),
            pltpu.VMEM((Dh, Dh), _F32),
            pltpu.SMEM((S, D), _BF16),
        ],
        compiler_params=pltpu.CompilerParams(vmem_limit_bytes=64 * 1024 * 1024),
    )(A_x.reshape(1, D), B_w_r.reshape(NC, _LANES), A_k_cache, A_v_cache, A_wq, A_wo,
      B_w_gate, B_w_up, B_w_down)
    return out.reshape(B, Sq, D)
```

```python
import jax
import jax.numpy as jnp
from jax import lax
import jax.experimental.pallas as pl
import jax.experimental.pallas.tpu as pltpu

_F32 = jnp.float32
_BF16 = jnp.bfloat16
_LANES = 128
_SUB = 8


def _dot(a, b):
    return jnp.dot(a, b, preferred_element_type=_F32)


def _dot_nt(a, b):
    return lax.dot_general(a, b, (((1,), (1,)), ((), ())), preferred_element_type=_F32)


def _tree_sum(xs):
    xs = list(xs)
    while len(xs) > 1:
        nxt = [xs[i] + xs[i + 1] for i in range(0, len(xs) - 1, 2)]
        if len(xs) % 2:
            nxt.append(xs[-1])
        xs = nxt
    return xs[0]


@jax.jit
def pallas_parallel_sum__sliding_block_cached__moe_arch_mod__decode_kernel(
    A_x: jax.Array,
    A_k_cache: jax.Array,
    A_v_cache: jax.Array,
    A_wq: jax.Array,
    A_wo: jax.Array,
    B_x: jax.Array,
    B_w_r: jax.Array,
    B_w_gate: jax.Array,
    B_w_up: jax.Array,
    B_w_down: jax.Array,
):
    del B_x
    B, Sq, D = A_x.shape
    Hq, Dh = 32, 128
    Hkv, Sk = A_k_cache.shape[1], A_k_cache.shape[2]
    W = min(4096, max(256, Sk // 4))
    rep = Hq // Hkv
    F = B_w_gate.shape[1]
    assert B == 1 and Sq == 1 and Hkv == 8 and Dh == _LANES and D % _LANES == 0
    R = _SUB
    scale = Dh ** -0.5
    G = rep * Dh
    NC = D // _LANES

    side = [(0, 256, "start", "wq"), (256, 288, "wq", "k4"), (544, 288, "k4", "wg")]
    S = side[-1][0] + side[-1][1]
    wo_mxu = [(S, 2048 - S), (2048, 1024), (3072, 512), (3584, 256)]
    wo_vpu = [(3840, 128), (3968, 64), (4032, 32), (4064, 32)]
    vpu_base = wo_vpu[0][0]
    n_mxu_heads = vpu_base // Dh
    assert n_mxu_heads * Dh == vpu_base
    n_copies = 3 + 2 * Hkv + 3 + len(wo_mxu) + len(wo_vpu) + 2 * len(side)

    def kernel(*refs):
        pl.run_scoped(lambda sems: body(*refs, sems),
                      pltpu.SemaphoreType.DMA((n_copies,)))

    def body(x_hbm, wr_hbm, k_hbm, v_hbm, wq_hbm, wo_hbm, wg_hbm, wu_hbm, wd_hbm,
             o_ref,
             xb, wrb, kb, vb, wqb, wob, wgb, wub, wdb, coef_ref, stage, sems):
        copies = {}

        def add(name, src, dst):
            copies[name] = pltpu.make_async_copy(src, dst, sems.at[len(copies)])

        add("wq", wq_hbm, wqb)
        add("x", x_hbm, xb)
        add("wr", wr_hbm, wrb)
        for h in range(Hkv):
            add("k%d" % h, k_hbm.at[0, h, pl.ds(Sk - W, W)], kb.at[h])
            add("v%d" % h, v_hbm.at[0, h, pl.ds(Sk - W, W)], vb.at[h])
        add("wg", wg_hbm, wgb)
        add("wu", wu_hbm, wub)
        add("wd", wd_hbm, wdb)
        for (r0, n) in wo_mxu + wo_vpu:
            add("wo%d" % r0, wo_hbm.at[pl.ds(r0, n)], wob.at[pl.ds(r0, n)])
        main = list(copies)
        for (r0, n, _, _) in side:
            add("h2s%d" % r0, wo_hbm.at[pl.ds(r0, n)], stage.at[pl.ds(r0, n)])
            add("s2v%d" % r0, stage.at[pl.ds(r0, n)], wob.at[pl.ds(r0, n)])
        assert len(copies) == n_copies

        def side_step(event):
            for (r0, _, _, e_s2v) in side:
                if e_s2v == event:
                    copies["h2s%d" % r0].wait()
                    copies["s2v%d" % r0].start()
            for (r0, _, e_h2s, _) in side:
                if e_h2s == event:
                    copies["h2s%d" % r0].start()

        def wait(name):
            copies[name].wait()
            side_step(name)

        copies[main[0]].start()
        side_step("start")
        for name in main[1:]:
            copies[name].start()

        wait("wq")
        wait("x")
        wait("wr")
        x = xb[...].astype(_F32)
        m = jnp.mean(x, axis=-1, keepdims=True)
        xc = x - m
        var = jnp.mean(xc * xc, axis=-1, keepdims=True)
        xn = xc / jnp.sqrt(var + 1e-5)
        xn = xn.astype(_BF16).astype(_F32)
        xn8 = jnp.broadcast_to(xn, (R, D)).astype(_BF16)
        wr = wrb[...].astype(_F32)
        racc = xn[:, 0:_LANES] * wr[0:1, :]
        for j in range(1, NC):
            racc = racc + xn[:, j * _LANES:(j + 1) * _LANES] * wr[j:j + 1, :]
        r = jnp.sum(racc, axis=-1, keepdims=True)
        r_sel = jax.nn.sigmoid(r)

        row = lax.broadcasted_iota(jnp.int32, (R, Dh), 0)

        q8 = _dot(xn8, wqb[...])

        lhs_o = []
        for h in range(Hkv):
            qh = q8[:, h * G:h * G + Dh]
            for j in range(1, rep):
                qh = jnp.where(row == j, q8[:, h * G + j * Dh:h * G + (j + 1) * Dh], qh)
            qh = qh.astype(_BF16)
            wait("k%d" % h)
            s = _dot_nt(qh, kb[h]) * scale
            mx = jnp.max(s, axis=-1, keepdims=True)
            p = jnp.exp(s - mx)
            l = jnp.sum(p, axis=-1, keepdims=True)
            wait("v%d" % h)
            oh = _dot(p.astype(_BF16), vb[h]) / l
            for j in range(rep):
                if h * rep + j < n_mxu_heads:
                    lhs_o.append(jnp.where(row == j, oh, 0.0).astype(_BF16))
                else:
                    o_row = oh[j:j + 1, :].astype(_BF16).astype(_F32)
                    c0 = (h * rep + j) * Dh - vpu_base
                    coef_ref[pl.ds(c0, Dh), :] = jnp.broadcast_to(o_row, (Dh, Dh)).T
        lo = jnp.concatenate(lhs_o, axis=1)

        wait("wg")
        g = _dot(xn8, wgb[...])
        wait("wu")
        u = _dot(xn8, wub[...])
        hh = (g * jax.nn.sigmoid(g) * u).astype(_BF16)
        wait("wd")
        y = _dot(hh, wdb[...]) * r_sel
        row_d = lax.broadcasted_iota(jnp.int32, (R, D), 0)
        acc = jnp.where(row_d == 0, (x + xn) + y, 0.0)

        for (r0, n) in wo_mxu:
            wait("wo%d" % r0)
            if r0 == S:
                for (s0, _, _, _) in side:
                    copies["s2v%d" % s0].wait()
                r0, n = 0, S + n
            acc = acc + _dot(lo[:, r0:r0 + n], wob[pl.ds(r0, n), :])
        accs = [acc[:, c * _LANES:(c + 1) * _LANES] for c in range(NC)]
        for (r0, n) in wo_vpu:
            cf = [coef_ref[pl.ds(r0 - vpu_base + i, _SUB), :] for i in range(0, n, _SUB)]
            wait("wo%d" % r0)
            w = wob[pl.ds(r0, n), :].astype(_F32)
            for c in range(NC):
                prods = [w[i * _SUB:(i + 1) * _SUB, c * _LANES:(c + 1) * _LANES] * cf[i]
                         for i in range(n // _SUB)]
                accs[c] = accs[c] + _tree_sum(prods)
        res = jnp.sum(jnp.concatenate(accs, axis=1), axis=0, keepdims=True)
        o_ref[...] = res.astype(o_ref.dtype)

    any_spec = pl.BlockSpec(memory_space=pl.ANY)
    out = pl.pallas_call(
        kernel,
        out_shape=jax.ShapeDtypeStruct((1, D), A_x.dtype),
        in_specs=[any_spec] * 9,
        out_specs=pl.BlockSpec(memory_space=pltpu.VMEM),
        scratch_shapes=[
            pltpu.VMEM((1, D), _BF16),
            pltpu.VMEM((NC, _LANES), _BF16),
            pltpu.VMEM((Hkv, W, Dh), _BF16),
            pltpu.VMEM((Hkv, W, Dh), _BF16),
            pltpu.VMEM((D, Hq * Dh), _BF16),
            pltpu.VMEM((Hq * Dh, D), _BF16),
            pltpu.VMEM((D, F), _BF16),
            pltpu.VMEM((D, F), _BF16),
            pltpu.VMEM((F, D), _BF16),
            pltpu.VMEM((Hq * Dh - vpu_base, Dh), _F32),
            pltpu.SMEM((S, D), _BF16),
        ],
        compiler_params=pltpu.CompilerParams(vmem_limit_bytes=64 * 1024 * 1024),
    )(A_x.reshape(1, D), B_w_r.reshape(NC, _LANES), A_k_cache, A_v_cache, A_wq, A_wo,
      B_w_gate, B_w_up, B_w_down)
    return out.reshape(B, Sq, D)
```

```python
import jax
import jax.numpy as jnp
from jax import lax
import jax.experimental.pallas as pl
import jax.experimental.pallas.tpu as pltpu

_F32 = jnp.float32
_BF16 = jnp.bfloat16
_LANES = 128
_SUB = 8


def _dot(a, b):
    return jnp.dot(a, b, preferred_element_type=_F32)


def _dot_nt(a, b):
    return lax.dot_general(a, b, (((1,), (1,)), ((), ())), preferred_element_type=_F32)


def _rnd(a):
    return a.astype(_BF16).astype(_F32)


def _tree_sum(xs):
    xs = list(xs)
    while len(xs) > 1:
        nxt = [xs[i] + xs[i + 1] for i in range(0, len(xs) - 1, 2)]
        if len(xs) % 2:
            nxt.append(xs[-1])
        xs = nxt
    return xs[0]


@jax.jit
def pallas_parallel_sum__sliding_block_cached__moe_arch_mod__decode_kernel(
    A_x: jax.Array,
    A_k_cache: jax.Array,
    A_v_cache: jax.Array,
    A_wq: jax.Array,
    A_wo: jax.Array,
    B_x: jax.Array,
    B_w_r: jax.Array,
    B_w_gate: jax.Array,
    B_w_up: jax.Array,
    B_w_down: jax.Array,
):
    del B_x
    B, Sq, D = A_x.shape
    Hq, Dh = 32, 128
    Hkv, Sk = A_k_cache.shape[1], A_k_cache.shape[2]
    W = min(4096, max(256, Sk // 4))
    rep = Hq // Hkv
    F = B_w_gate.shape[1]
    assert (B, Sq, D, Hkv, W, F) == (1, 1, 512, 8, 4096, 1792)
    R = _SUB
    G = rep * Dh
    NC = D // _LANES

    GQ, Q_ROWS, Q_COLS = 8, 8, 2048
    NB, KV_ROWS = 4, 128
    GF, F_ROWS, D_ROWS = 4, 8, 32
    KB = W // NB
    issue_after = {"k1": "q0", "k2": "q1", "k3": "k0", "v0": "k1", "v1": "k2", "v2": "k3",
                   "v3": "v0", "wg": "v2", "wu": "v3", "wd": "wg"}
    WO_ISSUE = "wu"
    ticks = ["q0", "q1", "k0", "k1", "k2", "k3", "v0", "v1", "v2", "v3", "wg", "wu", "wd", "wd"]
    S_ROWS, S_AHEAD = 64, 4
    n_side = len(ticks)
    S = n_side * S_ROWS
    side_use = {"wd": (0, 10), "wo0": (10, 12), "wo1": (12, 14)}
    wo_mxu = [(S, 2048 - S), (2048, 1024), (3072, 512), (3584, 256)]
    wo_vpu = [(3840, 128), (3968, 64), (4032, 32), (4064, 32)]
    vpu_base = wo_vpu[0][0]
    n_mxu_heads = vpu_base // Dh
    n_groups = 3 + 2 * NB + 3 + len(wo_mxu) + len(wo_vpu) + 2 * n_side

    def kernel(*refs):
        pl.run_scoped(lambda sems: body(*refs, sems),
                      pltpu.SemaphoreType.DMA((n_groups,)))

    def body(x_hbm, wr_hbm, k_hbm, v_hbm, wq_hbm, wo_hbm, wg_hbm, wu_hbm, wd_hbm,
             o_ref,
             xb, wrb, kb, vb, wqb, wob, wgb, wub, wdb, coef_ref, stage, sems):
        groups = {}
        main = []

        def add(name, src, dst, is_main=True):
            lst = groups.setdefault(name, [])
            c = pltpu.make_async_copy(src, dst, sems.at[list(groups).index(name)])
            lst.append(c)
            if is_main:
                main.append((name, c))

        def add_rows(name, src, dst, r, n):
            add(name, src.at[:, pl.ds(r, n)], dst.at[:, pl.ds(r, n)])

        q_reg = D // GQ
        for r in range(0, q_reg, Q_ROWS):
            for c0 in range(0, Hq * Dh, Q_COLS):
                sl = (slice(None), pl.ds(r, Q_ROWS), pl.ds(c0, Q_COLS))
                add("q%d" % (2 * r // q_reg), wq_hbm.at[sl], wqb.at[sl])
            if r == 0:
                add("x", x_hbm, xb)
                add("x", wr_hbm, wrb)
        for nm, src, dst in (("k", k_hbm, kb), ("v", v_hbm, vb)):
            for r in range(0, W, KV_ROWS):
                add("%s%d" % (nm, r // KB),
                    src.at[0, :, pl.ds(Sk - W + r, KV_ROWS)], dst.at[:, pl.ds(r, KV_ROWS)])
        for r in range(0, D // GF, F_ROWS):
            add_rows("wg", wg_hbm, wgb, r, F_ROWS)
        for r in range(0, D // GF, F_ROWS):
            add_rows("wu", wu_hbm, wub, r, F_ROWS)
        for r in range(0, F // GF, D_ROWS):
            add_rows("wd", wd_hbm, wdb, r, D_ROWS)
        for i, (r0, n) in enumerate(wo_mxu + wo_vpu):
            add("wo%d" % i, wo_hbm.at[pl.ds(r0, n)], wob.at[pl.ds(r0, n)])
            issue_after["wo%d" % i] = WO_ISSUE
        for i in range(n_side):
            rows = pl.ds(i * S_ROWS, S_ROWS)
            add("h2s%d" % i, wo_hbm.at[rows], stage.at[rows], False)
            add("s2v%d" % i, stage.at[rows], wob.at[rows], False)
        assert len(groups) == n_groups

        def wait_group(name):
            for c in groups[name]:
                c.wait()

        def wait(name):
            wait_group(name)
            for g_name, c in main:
                if issue_after.get(g_name) == name:
                    c.start()
            for i in range(n_side):
                if ticks[i] == name:
                    wait_group("h2s%d" % i)
                    groups["s2v%d" % i][0].start()
                    if i + S_AHEAD < n_side:
                        groups["h2s%d" % (i + S_AHEAD)][0].start()

        entry = [c for g_name, c in main if g_name not in issue_after]
        entry[0].start()
        for i in range(S_AHEAD):
            groups["h2s%d" % i][0].start()
        for c in entry[1:]:
            c.start()

        wait("x")
        x = xb[...].astype(_F32)
        m = jnp.mean(x, axis=-1, keepdims=True)
        xc = x - m
        var = jnp.mean(xc * xc, axis=-1, keepdims=True)
        eps = _rnd(jnp.full((1, 1), 1e-5, _F32))
        den = _rnd(jnp.sqrt(_rnd(_rnd(var) + eps)))
        xn = _rnd(_rnd(x - _rnd(m)) / den)
        xn8 = jnp.broadcast_to(xn, (R, D)).astype(_BF16)
        wr = wrb[...].astype(_F32)
        racc = xn[:, 0:_LANES] * wr[0:1, :]
        for j in range(1, NC):
            racc = racc + xn[:, j * _LANES:(j + 1) * _LANES] * wr[j:j + 1, :]
        r = _rnd(jnp.sum(racc, axis=-1, keepdims=True))
        r_sel = _rnd(jax.nn.sigmoid(r))
        scale = _rnd(jnp.full((1, 1), Dh ** -0.5, _F32))
        row = lax.broadcasted_iota(jnp.int32, (R, Dh), 0)

        wait("q0")
        wait("q1")
        q8 = _dot(xn8, wqb[...].reshape(D, Hq * Dh))
        qs = []
        for h in range(Hkv):
            qh = q8[:, h * G:h * G + Dh]
            for j in range(1, rep):
                qh = jnp.where(row == j, q8[:, h * G + j * Dh:h * G + (j + 1) * Dh], qh)
            qs.append(qh.astype(_BF16))

        s = [[] for _ in range(Hkv)]
        for b in range(NB):
            wait("k%d" % b)
            for h in range(Hkv):
                s[h].append(_rnd(_rnd(_dot_nt(qs[h], kb[h, pl.ds(b * KB, KB), :])) * scale))
        ps, ls = [], []
        for h in range(Hkv):
            sh = jnp.concatenate(s[h], axis=1)
            mx = jnp.max(sh, axis=-1, keepdims=True)
            p = jnp.exp(_rnd(sh - mx)).astype(_BF16)
            ps.append(p)
            ls.append(jnp.sum(p.astype(_F32), axis=-1, keepdims=True))
        pv = [None] * Hkv
        for b in range(NB):
            wait("v%d" % b)
            for h in range(Hkv):
                t = _dot(ps[h][:, b * KB:(b + 1) * KB], vb[h, pl.ds(b * KB, KB), :])
                pv[h] = t if pv[h] is None else pv[h] + t
        lhs_o = []
        for h in range(Hkv):
            oh = pv[h] / ls[h]
            for j in range(rep):
                if h * rep + j < n_mxu_heads:
                    lhs_o.append(jnp.where(row == j, oh, 0.0).astype(_BF16))
                else:
                    c0 = (h * rep + j) * Dh - vpu_base
                    coef_ref[pl.ds(c0, Dh), :] = jnp.broadcast_to(_rnd(oh[j:j + 1, :]), (Dh, Dh)).T
        lo = jnp.concatenate(lhs_o, axis=1)

        def wo_dot(r0, n):
            return _dot(lo[:, r0:r0 + n], wob[pl.ds(r0, n), :])

        def use_side(name, acc):
            if name not in side_use:
                return acc
            i0, i1 = side_use[name]
            for i in range(i0, i1):
                wait_group("s2v%d" % i)
            return acc + wo_dot(i0 * S_ROWS, (i1 - i0) * S_ROWS)

        wait("wg")
        g = _rnd(_dot(xn8, wgb[...].reshape(D, F)))
        g = _rnd(g * jax.nn.sigmoid(g))
        wait("wu")
        u = _rnd(_dot(xn8, wub[...].reshape(D, F)))
        hh = (g * u).astype(_BF16)
        wait("wd")
        y = _rnd(_dot(hh, wdb[...].reshape(F, D))) * r_sel
        row_d = lax.broadcasted_iota(jnp.int32, (R, D), 0)
        acc = jnp.where(row_d == 0, (x + xn) + y, 0.0)
        acc = use_side("wd", acc)

        for i, (r0, n) in enumerate(wo_mxu):
            wait("wo%d" % i)
            acc = use_side("wo%d" % i, acc + wo_dot(r0, n))
        accs = [acc[:, c * _LANES:(c + 1) * _LANES] for c in range(NC)]
        for i, (r0, n) in enumerate(wo_vpu):
            cf = [coef_ref[pl.ds(r0 - vpu_base + t, _SUB), :] for t in range(0, n, _SUB)]
            wait("wo%d" % (len(wo_mxu) + i))
            w = wob[pl.ds(r0, n), :].astype(_F32)
            for c in range(NC):
                prods = [w[t * _SUB:(t + 1) * _SUB, c * _LANES:(c + 1) * _LANES] * cf[t]
                         for t in range(n // _SUB)]
                accs[c] = accs[c] + _tree_sum(prods)
        res = jnp.sum(jnp.concatenate(accs, axis=1), axis=0, keepdims=True)
        o_ref[...] = res.astype(o_ref.dtype)

    any_spec = pl.BlockSpec(memory_space=pl.ANY)
    out = pl.pallas_call(
        kernel,
        out_shape=jax.ShapeDtypeStruct((1, D), A_x.dtype),
        in_specs=[any_spec] * 9,
        out_specs=pl.BlockSpec(memory_space=pltpu.VMEM),
        scratch_shapes=[
            pltpu.VMEM((1, D), _BF16),
            pltpu.VMEM((NC, _LANES), _BF16),
            pltpu.VMEM((Hkv, W, Dh), _BF16),
            pltpu.VMEM((Hkv, W, Dh), _BF16),
            pltpu.VMEM((GQ, D // GQ, Hq * Dh), _BF16),
            pltpu.VMEM((Hq * Dh, D), _BF16),
            pltpu.VMEM((GF, D // GF, F), _BF16),
            pltpu.VMEM((GF, D // GF, F), _BF16),
            pltpu.VMEM((GF, F // GF, D), _BF16),
            pltpu.VMEM((Hq * Dh - vpu_base, Dh), _F32),
            pltpu.SMEM((S, D), _BF16),
        ],
        compiler_params=pltpu.CompilerParams(vmem_limit_bytes=64 * 1024 * 1024),
    )(A_x.reshape(1, D), B_w_r.reshape(NC, _LANES), A_k_cache, A_v_cache,
      A_wq.reshape(GQ, D // GQ, Hq * Dh), A_wo,
      B_w_gate.reshape(GF, D // GF, F), B_w_up.reshape(GF, D // GF, F),
      B_w_down.reshape(GF, F // GF, D))
    return out.reshape(B, Sq, D)
```

```python
import jax
import jax.numpy as jnp
from jax import lax
import jax.experimental.pallas as pl
import jax.experimental.pallas.tpu as pltpu

_F32 = jnp.float32
_BF16 = jnp.bfloat16
_LANES = 128
_SUB = 8


def _dot(a, b):
    return jnp.dot(a, b, preferred_element_type=_F32)


def _dot_nt(a, b):
    return lax.dot_general(a, b, (((1,), (1,)), ((), ())), preferred_element_type=_F32)


def _rnd(a):
    return a.astype(_BF16).astype(_F32)


def _tree_sum(xs):
    xs = list(xs)
    while len(xs) > 1:
        nxt = [xs[i] + xs[i + 1] for i in range(0, len(xs) - 1, 2)]
        if len(xs) % 2:
            nxt.append(xs[-1])
        xs = nxt
    return xs[0]


@jax.jit
def pallas_parallel_sum__sliding_block_cached__moe_arch_mod__decode_kernel(
    A_x: jax.Array,
    A_k_cache: jax.Array,
    A_v_cache: jax.Array,
    A_wq: jax.Array,
    A_wo: jax.Array,
    B_x: jax.Array,
    B_w_r: jax.Array,
    B_w_gate: jax.Array,
    B_w_up: jax.Array,
    B_w_down: jax.Array,
):
    del B_x
    B, Sq, D = A_x.shape
    Hq, Dh = 32, 128
    Hkv, Sk = A_k_cache.shape[1], A_k_cache.shape[2]
    W = min(4096, max(256, Sk // 4))
    rep = Hq // Hkv
    F = B_w_gate.shape[1]
    assert (B, Sq, D, Hkv, W, F) == (1, 1, 512, 8, 4096, 1792)
    R = _SUB
    G = rep * Dh
    NC = D // _LANES

    AHEAD = 112
    HEAD, LAST = 40, 44
    GQ, GF = 8, 4
    NB = 8
    KB = W // NB
    GO = Hkv - 1
    tail_mxu = [(0, 256)]
    tail_vpu = [(256, 128), (384, 64), (448, 32), (480, 32)]
    v0 = tail_vpu[0][0]
    n_mxu_heads = GO * rep + v0 // Dh
    n_groups = 2 + 2 * NB + 3 + rep + len(tail_mxu) + len(tail_vpu)

    def kernel(*refs):
        pl.run_scoped(lambda sems: body(*refs, sems),
                      pltpu.SemaphoreType.DMA((n_groups,)))

    def body(x_hbm, wr_hbm, k_hbm, v_hbm, wq_hbm, wo_hbm, wg_hbm, wu_hbm, wd_hbm,
             o_ref,
             xb, wrb, kb, vb, wqb, wob, wgb, wub, wdb, coef_ref, sems):
        groups = {}
        stream = []

        def group(name, *regions):
            groups[name] = (sems.at[len(groups)], regions)

        def add(name, src, dst, *idx):
            stream.append((name, src.at[idx], dst.at[idx]))

        group("q", wqb)
        group("x", xb, wrb)
        for r in range(0, D // GQ, 8):
            for c in range(0, Hq * Dh, 2048):
                for g in range(GQ):
                    add("q", wq_hbm, wqb, pl.ds(g * (D // GQ) + r, 8), pl.ds(c, 2048))
            if r == 0:
                stream.append(("x", x_hbm, xb))
                stream.append(("x", wr_hbm, wrb))
        for nm, src, dst in (("k", k_hbm, kb), ("v", v_hbm, vb)):
            win = src.at[0, :, pl.ds(Sk - W, W)]
            for b in range(NB):
                group("%s%d" % (nm, b), dst.at[:, pl.ds(b * KB, KB)])
                for r in range(b * KB, (b + 1) * KB, 128):
                    for h in range(Hkv):
                        add("%s%d" % (nm, b), win, dst, h, pl.ds(r, 128))
        for nm, src, dst, n in (("wg", wg_hbm, wgb, 8), ("wu", wu_hbm, wub, 8),
                                ("wd", wd_hbm, wdb, 32)):
            group(nm, dst)
            reg = dst.shape[0] // GF
            for r in range(0, reg, n):
                for g in range(GF):
                    add(nm, src, dst, pl.ds(g * reg + r, n))
        for j in range(rep):
            group("o%d" % j, wob.at[pl.ds(0, GO), pl.ds(j * Dh, Dh)])
            for r in range(j * Dh, (j + 1) * Dh, 32):
                for h in range(GO):
                    add("o%d" % j, wo_hbm, wob, h, pl.ds(r, 32))
        for i, (r0, n) in enumerate(tail_mxu + tail_vpu):
            group("t%d" % i, wob.at[GO, pl.ds(r0, n)])
            for r in range(r0, r0 + n, 16):
                add("t%d" % i, wo_hbm, wob, GO, pl.ds(r, 16))
        assert len(groups) == n_groups
        n_stream = len(stream)
        last = {name: i for i, (name, _, _) in enumerate(stream)}
        issued = [0]

        def issue_to(n):
            for i in range(issued[0], min(n, n_stream)):
                name, src, dst = stream[i]
                prio = 1 if (i < HEAD or i >= n_stream - LAST) else (i + 1) % 2
                pltpu.make_async_copy(src, dst, groups[name][0]).start(
                    priority=0 if name == "x" else prio)
                issued[0] = i + 1

        def wait(name):
            issue_to(last[name] + 1 + AHEAD)
            sem, regions = groups[name]
            for reg in regions:
                pltpu.make_async_copy(reg, reg, sem).wait()

        wait("x")
        x = xb[...].astype(_F32)
        m = jnp.mean(x, axis=-1, keepdims=True)
        xc = x - m
        var = jnp.mean(xc * xc, axis=-1, keepdims=True)
        eps = _rnd(jnp.full((1, 1), 1e-5, _F32))
        den = _rnd(jnp.sqrt(_rnd(_rnd(var) + eps)))
        xn = _rnd(_rnd(x - _rnd(m)) / den)
        xn8 = jnp.broadcast_to(xn, (R, D)).astype(_BF16)
        wr = wrb[...].astype(_F32)
        racc = xn[:, 0:_LANES] * wr[0:1, :]
        for j in range(1, NC):
            racc = racc + xn[:, j * _LANES:(j + 1) * _LANES] * wr[j:j + 1, :]
        r_sel = _rnd(jax.nn.sigmoid(_rnd(jnp.sum(racc, axis=-1, keepdims=True))))
        scale = _rnd(jnp.full((1, 1), Dh ** -0.5, _F32))
        row = lax.broadcasted_iota(jnp.int32, (R, Dh), 0)

        wait("q")
        qs = []
        half = Hkv // 2
        for part in range(2):
            issue_to(issued[0] + 8 * part)
            q8 = _dot(xn8, wqb[:, pl.ds(part * half * G, half * G)])
            for h in range(half):
                qh = q8[:, h * G:h * G + Dh]
                for j in range(1, rep):
                    qh = jnp.where(row == j, q8[:, h * G + j * Dh:h * G + (j + 1) * Dh], qh)
                qs.append(qh.astype(_BF16))

        s = [[] for _ in range(Hkv)]
        for b in range(NB):
            wait("k%d" % b)
            for h in range(Hkv):
                s[h].append(_rnd(_rnd(_dot_nt(qs[h], kb[h, pl.ds(b * KB, KB), :])) * scale))
        issue_to(issued[0] + 8)
        ps, ls = [], []
        for h in range(Hkv):
            sh = jnp.concatenate(s[h], axis=1)
            mx = jnp.max(sh, axis=-1, keepdims=True)
            p = jnp.exp(_rnd(sh - mx)).astype(_BF16)
            ps.append(p)
            ls.append(jnp.sum(p.astype(_F32), axis=-1, keepdims=True))
        pv = [None] * Hkv
        for b in range(NB):
            wait("v%d" % b)
            for h in range(Hkv):
                t = _dot(ps[h][:, b * KB:(b + 1) * KB], vb[h, pl.ds(b * KB, KB), :])
                pv[h] = t if pv[h] is None else pv[h] + t
        lhs_o = []
        for h in range(Hkv):
            oh = pv[h] / ls[h]
            for j in range(rep):
                if h * rep + j < n_mxu_heads:
                    lhs_o.append(jnp.where(row == j, oh, 0.0).astype(_BF16))
                else:
                    c0 = j * Dh - v0
                    coef_ref[pl.ds(c0, Dh), :] = jnp.broadcast_to(_rnd(oh[j:j + 1, :]), (Dh, Dh)).T

        wait("wg")
        gt = _rnd(_dot(xn8, wgb[...]))
        gt = _rnd(gt * jax.nn.sigmoid(gt))
        wait("wu")
        up = _rnd(_dot(xn8, wub[...]))
        hh = (gt * up).astype(_BF16)
        wait("wd")
        y = _rnd(_dot(hh, wdb[...])) * r_sel
        row_d = lax.broadcasted_iota(jnp.int32, (R, D), 0)
        acc = jnp.where(row_d == 0, (x + xn) + y, 0.0)

        for j in range(rep):
            wait("o%d" % j)
            lhs = jnp.concatenate([lhs_o[h * rep + j] for h in range(GO)], axis=1)
            acc = acc + _dot(lhs, wob[pl.ds(0, GO), pl.ds(j * Dh, Dh), :].reshape(GO * Dh, D))
        for i, (r0, n) in enumerate(tail_mxu):
            wait("t%d" % i)
            lhs = jnp.concatenate(lhs_o[GO * rep + r0 // Dh:GO * rep + (r0 + n) // Dh], axis=1)
            acc = acc + _dot(lhs, wob[GO, pl.ds(r0, n), :])
        accs = [acc[:, c * _LANES:(c + 1) * _LANES] for c in range(NC)]
        for i, (r0, n) in enumerate(tail_vpu):
            cf = [coef_ref[pl.ds(r0 - v0 + t, _SUB), :] for t in range(0, n, _SUB)]
            wait("t%d" % (len(tail_mxu) + i))
            w = wob[GO, pl.ds(r0, n), :].astype(_F32)
            for c in range(NC):
                prods = [w[t * _SUB:(t + 1) * _SUB, c * _LANES:(c + 1) * _LANES] * cf[t]
                         for t in range(n // _SUB)]
                accs[c] = accs[c] + _tree_sum(prods)
        assert issued[0] == n_stream
        res = jnp.sum(jnp.concatenate(accs, axis=1), axis=0, keepdims=True)
        o_ref[...] = res.astype(o_ref.dtype)

    any_spec = pl.BlockSpec(memory_space=pl.ANY)
    out = pl.pallas_call(
        kernel,
        out_shape=jax.ShapeDtypeStruct((1, D), A_x.dtype),
        in_specs=[any_spec] * 9,
        out_specs=pl.BlockSpec(memory_space=pltpu.VMEM),
        scratch_shapes=[
            pltpu.VMEM((1, D), _BF16),
            pltpu.VMEM((NC, _LANES), _BF16),
            pltpu.VMEM((Hkv, W, Dh), _BF16),
            pltpu.VMEM((Hkv, W, Dh), _BF16),
            pltpu.VMEM((D, Hq * Dh), _BF16),
            pltpu.VMEM((Hkv, G, D), _BF16),
            pltpu.VMEM((D, F), _BF16),
            pltpu.VMEM((D, F), _BF16),
            pltpu.VMEM((F, D), _BF16),
            pltpu.VMEM((G - v0, Dh), _F32),
        ],
        compiler_params=pltpu.CompilerParams(vmem_limit_bytes=64 * 1024 * 1024),
    )(A_x.reshape(1, D), B_w_r.reshape(NC, _LANES), A_k_cache, A_v_cache,
      A_wq, A_wo.reshape(Hkv, G, D), B_w_gate, B_w_up, B_w_down)
    return out.reshape(B, Sq, D)
```

```python
import jax
import jax.numpy as jnp
from jax import lax
import jax.experimental.pallas as pl
import jax.experimental.pallas.tpu as pltpu

_F32 = jnp.float32
_BF16 = jnp.bfloat16
_LANES = 128
_SUB = 8


def _dot(a, b):
    return jnp.dot(a, b, preferred_element_type=_F32)


def _dot_nt(a, b):
    return lax.dot_general(a, b, (((1,), (1,)), ((), ())), preferred_element_type=_F32)


def _rnd(a):
    return a.astype(_BF16).astype(_F32)


def _tree_sum(xs):
    xs = list(xs)
    while len(xs) > 1:
        nxt = [xs[i] + xs[i + 1] for i in range(0, len(xs) - 1, 2)]
        if len(xs) % 2:
            nxt.append(xs[-1])
        xs = nxt
    return xs[0]


def _hop(items, regions):
    n = len(items) // regions
    assert n * regions == len(items)
    return [items[g * n + i] for i in range(n) for g in range(regions)]


@jax.jit
def pallas_parallel_sum__sliding_block_cached__moe_arch_mod__decode_kernel(
    A_x: jax.Array,
    A_k_cache: jax.Array,
    A_v_cache: jax.Array,
    A_wq: jax.Array,
    A_wo: jax.Array,
    B_x: jax.Array,
    B_w_r: jax.Array,
    B_w_gate: jax.Array,
    B_w_up: jax.Array,
    B_w_down: jax.Array,
):
    del B_x
    B, Sq, D = A_x.shape
    Hq, Dh = 32, 128
    Hkv, Sk = A_k_cache.shape[1], A_k_cache.shape[2]
    W = min(4096, max(256, Sk // 4))
    rep = Hq // Hkv
    F = B_w_gate.shape[1]
    assert (B, Sq, D, Hkv, W, F) == (1, 1, 512, 8, 4096, 1792)
    R = _SUB
    G = rep * Dh
    NC = D // _LANES

    AHEAD = 108
    BUMP = 14
    HEAD, LAST = 20, 48
    GQ, GF = 8, 4
    NB = 8
    KB = W // NB
    FR = D // GF
    u_split = [(0, 96), (96, FR)]
    T0 = 3072
    tail_mxu = [(3072, 512, 32), (3584, 256, 16)]
    tail_vpu = [(3840, 128, 16), (3968, 64, 16), (4032, 32, 16), (4064, 32, 16)]
    v0 = tail_vpu[0][0]
    n_mxu_heads = v0 // Dh
    n_groups = 2 + 2 * NB + 1 + len(u_split) + len(tail_mxu) + len(tail_vpu) + 2

    def kernel(*refs):
        pl.run_scoped(lambda sems: body(*refs, sems),
                      pltpu.SemaphoreType.DMA((n_groups,)))

    def body(x_hbm, wr_hbm, k_hbm, v_hbm, wq_hbm, wo_hbm, wg_hbm, wu_hbm, wd_hbm,
             o_ref,
             xb, wrb, kb, vb, wqb, wob, wgb, wub, wdb, coef_ref, sems):
        groups = {}
        main, woven = [], []

        def group(name, *regions):
            groups[name] = (sems.at[len(groups)], regions)

        def piece(name, src, dst, *idx):
            return (name, src.at[idx], dst.at[idx])

        group("x", xb, wrb)
        group("q", wqb)
        for r, c in _hop([(r, c) for r in range(0, D, 8) for c in range(0, Hq * Dh, 2048)], GQ):
            main.append(piece("q", wq_hbm, wqb, pl.ds(r, 8), pl.ds(c, 2048)))
        for nm, src, dst in (("k", k_hbm, kb), ("v", v_hbm, vb)):
            win = src.at[0, :, pl.ds(Sk - W, W)]
            for b in range(NB):
                group("%s%d" % (nm, b), dst.at[:, pl.ds(b * KB, KB)])
                for r in range(b * KB, (b + 1) * KB, 128):
                    for h in range(Hkv):
                        main.append(piece("%s%d" % (nm, b), win, dst, h, pl.ds(r, 128)))
        group("wg", wgb)
        for r in _hop(list(range(0, D, 8)), GF):
            main.append(piece("wg", wg_hbm, wgb, pl.ds(r, 8)))
        for i, (lo, hi) in enumerate(u_split):
            group("wu%d" % i, wub.at[:, pl.ds(lo, hi - lo)])
            for r in range(lo, hi, 8):
                for g in range(GF):
                    main.append(piece("wu%d" % i, wu_hbm, wub, g, pl.ds(r, 8)))
        for i, (r0, n, rows) in enumerate(tail_mxu + tail_vpu):
            group("t%d" % i, wob.at[pl.ds(r0, n)])
            for r in range(r0, r0 + n, rows):
                main.append(piece("t%d" % i, wo_hbm, wob, pl.ds(r, rows)))
        group("wo", wob.at[pl.ds(0, T0)])
        for r in _hop(list(range(0, T0, 8)), GF):
            woven.append(piece("wo", wo_hbm, wob, pl.ds(r, 8)))
        group("wd", wdb)
        for r in _hop(list(range(0, F, 8)), GF):
            woven.append(piece("wd", wd_hbm, wdb, pl.ds(r, 8)))
        assert len(groups) == n_groups

        stream = []
        span = len(main) - HEAD - LAST
        n_w = 0
        for i, p in enumerate(main):
            stream.append(p + (1,))
            if i == 0:
                stream.append(("x", x_hbm, xb, 0))
                stream.append(("x", wr_hbm, wrb, 0))
            while n_w < len(woven) and n_w * span < (i - HEAD + 1) * len(woven):
                stream.append(woven[n_w] + (0,))
                n_w += 1
        assert n_w == len(woven)
        last = {p[0]: i for i, p in enumerate(stream)}
        issued = [0]

        def issue_to(n):
            for i in range(issued[0], min(n, len(stream))):
                name, src, dst, prio = stream[i]
                pltpu.make_async_copy(src, dst, groups[name][0]).start(priority=prio)
                issued[0] = i + 1

        def bump():
            issue_to(issued[0] + BUMP)

        def wait(name, ahead=AHEAD):
            issue_to(last[name] + 1 + ahead)
            sem, regions = groups[name]
            for reg in regions:
                pltpu.make_async_copy(reg, reg, sem).wait()

        wait("x", 96)
        x = xb[...].astype(_F32)
        m = jnp.mean(x, axis=-1, keepdims=True)
        xc = x - m
        var = jnp.mean(xc * xc, axis=-1, keepdims=True)
        eps = _rnd(jnp.full((1, 1), 1e-5, _F32))
        den = _rnd(jnp.sqrt(_rnd(_rnd(var) + eps)))
        xn = _rnd(_rnd(x - _rnd(m)) / den)
        xn8f = jnp.broadcast_to(xn, (R, D))
        xn8 = xn8f.astype(_BF16)
        xu = [jnp.concatenate([xn8f[:, g * FR + lo:g * FR + hi] for g in range(GF)],
                              axis=1).astype(_BF16) for lo, hi in u_split]
        wr = wrb[...].astype(_F32)
        racc = xn[:, 0:_LANES] * wr[0:1, :]
        for j in range(1, NC):
            racc = racc + xn[:, j * _LANES:(j + 1) * _LANES] * wr[j:j + 1, :]
        r_sel = _rnd(jax.nn.sigmoid(_rnd(jnp.sum(racc, axis=-1, keepdims=True))))
        scale = _rnd(jnp.full((1, 1), Dh ** -0.5, _F32))
        row = lax.broadcasted_iota(jnp.int32, (R, Dh), 0)

        wait("q")
        qs = []
        half = Hkv // 2
        for part in range(2):
            if part:
                bump()
            q8 = _dot(xn8, wqb[:, pl.ds(part * half * G, half * G)])
            for h in range(half):
                qh = q8[:, h * G:h * G + Dh]
                for j in range(1, rep):
                    qh = jnp.where(row == j, q8[:, h * G + j * Dh:h * G + (j + 1) * Dh], qh)
                qs.append(qh.astype(_BF16))

        s = [[] for _ in range(Hkv)]
        for b in range(NB):
            wait("k%d" % b)
            for h in range(Hkv):
                s[h].append(_rnd(_rnd(_dot_nt(qs[h], kb[h, pl.ds(b * KB, KB), :])) * scale))
        bump()
        ps, ls = [], []
        for h in range(Hkv):
            sh = jnp.concatenate(s[h], axis=1)
            mx = jnp.max(sh, axis=-1, keepdims=True)
            p = jnp.exp(_rnd(sh - mx)).astype(_BF16)
            ps.append(p)
            ls.append(jnp.sum(p.astype(_F32), axis=-1, keepdims=True))
        pv = [None] * Hkv
        for b in range(NB):
            wait("v%d" % b)
            for h in range(Hkv):
                t = _dot(ps[h][:, b * KB:(b + 1) * KB], vb[h, pl.ds(b * KB, KB), :])
                pv[h] = t if pv[h] is None else pv[h] + t
        lhs_o = []
        for h in range(Hkv):
            oh = pv[h] / ls[h]
            for j in range(rep):
                if h * rep + j < n_mxu_heads:
                    lhs_o.append(jnp.where(row == j, oh, 0.0).astype(_BF16))
                else:
                    c0 = (h * rep + j) * Dh - v0
                    coef_ref[pl.ds(c0, Dh), :] = jnp.broadcast_to(_rnd(oh[j:j + 1, :]), (Dh, Dh)).T

        def wo_dot(r0, n):
            lhs = jnp.concatenate(lhs_o[r0 // Dh:(r0 + n) // Dh], axis=1)
            return _dot(lhs, wob[pl.ds(r0, n), :])

        row_d = lax.broadcasted_iota(jnp.int32, (R, D), 0)
        acc = jnp.where(row_d == 0, x + xn, 0.0)
        wait("wo", 0)
        for part in range(2):
            bump()
            acc = acc + wo_dot(part * (T0 // 2), T0 // 2)

        wait("wg")
        gt = _rnd(_dot(xn8, wgb[...]))
        gt = _rnd(gt * jax.nn.sigmoid(gt))
        up = None
        for i, (lo, hi) in enumerate(u_split):
            if i == len(u_split) - 1:
                wait("wd", 0)
            wait("wu%d" % i)
            t = _dot(xu[i], wub[:, pl.ds(lo, hi - lo), :].reshape(GF * (hi - lo), F))
            up = t if up is None else up + t
        hh = (gt * _rnd(up)).astype(_BF16)
        y = _rnd(_dot(hh, wdb[...])) * r_sel
        acc = acc + jnp.where(row_d == 0, y, 0.0)

        for i, (r0, n, _) in enumerate(tail_mxu):
            wait("t%d" % i)
            acc = acc + wo_dot(r0, n)
        accs = [acc[:, c * _LANES:(c + 1) * _LANES] for c in range(NC)]
        for i, (r0, n, _) in enumerate(tail_vpu):
            cf = [coef_ref[pl.ds(r0 - v0 + t, _SUB), :] for t in range(0, n, _SUB)]
            wait("t%d" % (len(tail_mxu) + i))
            w = wob[pl.ds(r0, n), :].astype(_F32)
            for c in range(NC):
                prods = [w[t * _SUB:(t + 1) * _SUB, c * _LANES:(c + 1) * _LANES] * cf[t]
                         for t in range(n // _SUB)]
                accs[c] = accs[c] + _tree_sum(prods)
        assert issued[0] == len(stream)
        res = jnp.sum(jnp.concatenate(accs, axis=1), axis=0, keepdims=True)
        o_ref[...] = res.astype(o_ref.dtype)

    any_spec = pl.BlockSpec(memory_space=pl.ANY)
    out = pl.pallas_call(
        kernel,
        out_shape=jax.ShapeDtypeStruct((1, D), A_x.dtype),
        in_specs=[any_spec] * 9,
        out_specs=pl.BlockSpec(memory_space=pltpu.VMEM),
        scratch_shapes=[
            pltpu.VMEM((1, D), _BF16),
            pltpu.VMEM((NC, _LANES), _BF16),
            pltpu.VMEM((Hkv, W, Dh), _BF16),
            pltpu.VMEM((Hkv, W, Dh), _BF16),
            pltpu.VMEM((D, Hq * Dh), _BF16),
            pltpu.VMEM((Hq * Dh, D), _BF16),
            pltpu.VMEM((D, F), _BF16),
            pltpu.VMEM((GF, FR, F), _BF16),
            pltpu.VMEM((F, D), _BF16),
            pltpu.VMEM((Hq * Dh - v0, Dh), _F32),
        ],
        compiler_params=pltpu.CompilerParams(vmem_limit_bytes=64 * 1024 * 1024),
    )(A_x.reshape(1, D), B_w_r.reshape(NC, _LANES), A_k_cache, A_v_cache,
      A_wq, A_wo, B_w_gate, B_w_up.reshape(GF, FR, F), B_w_down)
    return out.reshape(B, Sq, D)
```

```python
import jax
import jax.numpy as jnp
from jax import lax
import jax.experimental.pallas as pl
import jax.experimental.pallas.tpu as pltpu

_F32 = jnp.float32
_BF16 = jnp.bfloat16
_LANES = 128
_SUB = 8


def _dot(a, b):
    return jnp.dot(a, b, preferred_element_type=_F32)


def _dot_nt(a, b):
    return lax.dot_general(a, b, (((1,), (1,)), ((), ())), preferred_element_type=_F32)


def _rnd(a):
    return a.astype(_BF16).astype(_F32)


def _tree_sum(xs):
    xs = list(xs)
    while len(xs) > 1:
        nxt = [xs[i] + xs[i + 1] for i in range(0, len(xs) - 1, 2)]
        if len(xs) % 2:
            nxt.append(xs[-1])
        xs = nxt
    return xs[0]


def _rects(t0, t1, c):
    out = []
    if t0 % c:
        e = min(t1, (t0 // c + 1) * c)
        out.append((pl.ds(t0 // c * _SUB, _SUB), pl.ds(t0 % c * _LANES, (e - t0) * _LANES)))
        t0 = e
    if t1 // c > t0 // c:
        out.append((pl.ds(t0 // c * _SUB, (t1 // c - t0 // c) * _SUB), pl.ds(0, c * _LANES)))
        t0 = t1 // c * c
    if t1 > t0:
        out.append((pl.ds(t0 // c * _SUB, _SUB), pl.ds(0, (t1 - t0) * _LANES)))
    return out


def _cut(lo, hi, phase, size):
    cuts = [lo] + [t for t in range(lo + 1, hi) if t % size == phase % size] + [hi]
    return list(zip(cuts[:-1], cuts[1:]))


def _round_robin(parts):
    return [p[i] for i in range(max(map(len, parts))) for p in parts if i < len(p)]


def _hop(items, regions):
    n = -(-len(items) // regions)
    return _round_robin([items[g * n:(g + 1) * n] for g in range(regions)])


@jax.jit
def pallas_parallel_sum__sliding_block_cached__moe_arch_mod__decode_kernel(
    A_x: jax.Array,
    A_k_cache: jax.Array,
    A_v_cache: jax.Array,
    A_wq: jax.Array,
    A_wo: jax.Array,
    B_x: jax.Array,
    B_w_r: jax.Array,
    B_w_gate: jax.Array,
    B_w_up: jax.Array,
    B_w_down: jax.Array,
):
    del B_x
    B, Sq, D = A_x.shape
    Hq, Dh = 32, 128
    Hkv, Sk = A_k_cache.shape[1], A_k_cache.shape[2]
    W = min(4096, max(256, Sk // 4))
    rep = Hq // Hkv
    F = B_w_gate.shape[1]
    assert (B, Sq, D, Hkv, W, F) == (1, 1, 512, 8, 4096, 1792)
    R = _SUB
    G = rep * Dh
    NC = D // _LANES

    BIG, SMALL = 16, 4
    PH_A, PH_B = 14, 15
    AHEAD = 140
    BUMP = 20
    HEAD, LAST = 20, 48
    GQ, GF = 8, 4
    NB = 8
    KB = W // NB
    FR = D // GF
    u_split = [(0, 96), (96, FR)]
    T0 = 3072
    tail_mxu = [(3072, 512, 32), (3584, 256, 16)]
    tail_vpu = [(3840, 128, 16), (3968, 64, 16), (4032, 32, 16), (4064, 32, 16)]
    v0 = tail_vpu[0][0]
    n_mxu_heads = v0 // Dh
    n_groups = 2 + 2 * NB + 1 + len(u_split) + len(tail_mxu) + len(tail_vpu) + 2

    def kernel(*refs):
        pl.run_scoped(lambda sems: body(*refs, sems),
                      pltpu.SemaphoreType.DMA((n_groups,)))

    def body(x_hbm, wr_hbm, k_hbm, v_hbm, wq_hbm, wo_hbm, wg_hbm, wu_hbm, wd_hbm,
             o_ref,
             xb, wrb, kb, vb, wqb, wob, wgb, wub, wdb, coef_ref, sems):
        groups = {}
        main, woven = [], []

        def group(name, *regions):
            groups[name] = (sems.at[len(groups)], regions)

        def piece(name, src, dst, t0, t1):
            return [(name, src.at[idx], dst.at[idx])
                    for idx in _rects(t0, t1, dst.shape[1] // _LANES)]

        def tiles(ref, rows=None):
            return (ref.shape[0] if rows is None else rows) // _SUB * (ref.shape[1] // _LANES)

        group("x", xb, wrb)
        group("q", wqb)
        for a, b in _hop(_cut(0, tiles(wqb), PH_A, BIG), GQ):
            main.append(piece("q", wq_hbm, wqb, a, b))
        kv_bounds = [0] + [b * KB // _SUB + PH_A for b in range(1, NB)] + [W // _SUB]
        for nm, src, dst in (("k", k_hbm, kb), ("v", v_hbm, vb)):
            for b in range(NB):
                lo, hi = kv_bounds[b], kv_bounds[b + 1]
                group("%s%d" % (nm, b), dst.at[:, pl.ds(lo * _SUB, (hi - lo) * _SUB)])
                for a, e in _cut(lo, hi, PH_A, BIG):
                    for h in range(Hkv):
                        main.append(piece("%s%d" % (nm, b), src.at[0, h, pl.ds(Sk - W, W)],
                                          dst.at[h], a, e))
        group("wg", wgb)
        for a, b in _hop(_cut(0, tiles(wgb), PH_B, BIG), GF):
            main.append(piece("wg", wg_hbm, wgb, a, b))
        u_parts, u_regions = ([], []), ([], [])
        for g in range(GF):
            lo, hi = tiles(wub, g * FR), tiles(wub, (g + 1) * FR)
            cuts = _cut(lo, hi, PH_B, BIG)
            first = [c for c in cuts if c[0] < tiles(wub, g * FR + u_split[0][1])]
            mid = first[-1][1]
            u_parts[0].append(first)
            u_parts[1].append(cuts[len(first):])
            u_regions[0].extend(wub.at[idx] for idx in _rects(lo, mid, F // _LANES))
            u_regions[1].extend(wub.at[idx] for idx in _rects(mid, hi, F // _LANES))
        for i in range(2):
            group("wu%d" % i, *u_regions[i])
            for a, b in _round_robin(u_parts[i]):
                main.append(piece("wu%d" % i, wu_hbm, wub, a, b))
        for i, (r0, n, rows) in enumerate(tail_mxu + tail_vpu):
            group("t%d" % i, wob.at[pl.ds(r0, n)])
            for r in range(r0, r0 + n, rows):
                main.append(piece("t%d" % i, wo_hbm, wob, tiles(wob, r), tiles(wob, r + rows)))
        group("wo", wob.at[pl.ds(0, T0)])
        for a, b in _hop(_cut(0, tiles(wob, T0), PH_A, SMALL), GF):
            woven.append(piece("wo", wo_hbm, wob, a, b))
        group("wd", wdb)
        for a, b in _hop(_cut(0, tiles(wdb), 0, SMALL), GF):
            woven.append(piece("wd", wd_hbm, wdb, a, b))
        assert len(groups) == n_groups

        stream = []
        span = len(main) - HEAD - LAST
        n_w = 0
        for i, p in enumerate(main):
            stream.extend(c + (1,) for c in p)
            if i == 0:
                stream.append(("x", x_hbm, xb, 0))
                stream.append(("x", wr_hbm, wrb, 0))
            while n_w < len(woven) and n_w * span < (i - HEAD + 1) * len(woven):
                stream.extend(c + (0,) for c in woven[n_w])
                n_w += 1
        assert n_w == len(woven)
        last = {c[0]: i for i, c in enumerate(stream)}
        issued = [0]

        def issue_to(n):
            for i in range(issued[0], min(n, len(stream))):
                name, src, dst, prio = stream[i]
                pltpu.make_async_copy(src, dst, groups[name][0]).start(priority=prio)
                issued[0] = i + 1

        def bump():
            issue_to(issued[0] + BUMP)

        def wait(name, ahead=AHEAD):
            issue_to(last[name] + 1 + ahead)
            sem, regions = groups[name]
            for reg in regions:
                pltpu.make_async_copy(reg, reg, sem).wait()

        wait("x", 96)
        x = xb[...].astype(_F32)
        m = jnp.mean(x, axis=-1, keepdims=True)
        xc = x - m
        var = jnp.mean(xc * xc, axis=-1, keepdims=True)
        eps = _rnd(jnp.full((1, 1), 1e-5, _F32))
        den = _rnd(jnp.sqrt(_rnd(_rnd(var) + eps)))
        xn = _rnd(_rnd(x - _rnd(m)) / den)
        xn8f = jnp.broadcast_to(xn, (R, D))
        xn8 = xn8f.astype(_BF16)
        xu = [jnp.concatenate([xn8f[:, g * FR + lo:g * FR + hi] for g in range(GF)],
                              axis=1).astype(_BF16) for lo, hi in u_split]
        wr = wrb[...].astype(_F32)
        racc = xn[:, 0:_LANES] * wr[0:1, :]
        for j in range(1, NC):
            racc = racc + xn[:, j * _LANES:(j + 1) * _LANES] * wr[j:j + 1, :]
        r_sel = _rnd(jax.nn.sigmoid(_rnd(jnp.sum(racc, axis=-1, keepdims=True))))
        scale = _rnd(jnp.full((1, 1), Dh ** -0.5, _F32))
        row = lax.broadcasted_iota(jnp.int32, (R, Dh), 0)

        wait("q")
        qs = []
        half = Hkv // 2
        for part in range(2):
            if part:
                bump()
            q8 = _dot(xn8, wqb[:, pl.ds(part * half * G, half * G)])
            for h in range(half):
                qh = q8[:, h * G:h * G + Dh]
                for j in range(1, rep):
                    qh = jnp.where(row == j, q8[:, h * G + j * Dh:h * G + (j + 1) * Dh], qh)
                qs.append(qh.astype(_BF16))

        s = [[] for _ in range(Hkv)]
        for b in range(NB):
            wait("k%d" % b)
            for h in range(Hkv):
                s[h].append(_rnd(_rnd(_dot_nt(qs[h], kb[h, pl.ds(b * KB, KB), :])) * scale))
        bump()
        ps, ls = [], []
        for h in range(Hkv):
            sh = jnp.concatenate(s[h], axis=1)
            mx = jnp.max(sh, axis=-1, keepdims=True)
            p = jnp.exp(_rnd(sh - mx)).astype(_BF16)
            ps.append(p)
            ls.append(jnp.sum(p.astype(_F32), axis=-1, keepdims=True))
        pv = [None] * Hkv
        for b in range(NB):
            wait("v%d" % b)
            for h in range(Hkv):
                t = _dot(ps[h][:, b * KB:(b + 1) * KB], vb[h, pl.ds(b * KB, KB), :])
                pv[h] = t if pv[h] is None else pv[h] + t
        lhs_o = []
        for h in range(Hkv):
            oh = pv[h] / ls[h]
            for j in range(rep):
                if h * rep + j < n_mxu_heads:
                    lhs_o.append(jnp.where(row == j, oh, 0.0).astype(_BF16))
                else:
                    c0 = (h * rep + j) * Dh - v0
                    coef_ref[pl.ds(c0, Dh), :] = jnp.broadcast_to(_rnd(oh[j:j + 1, :]), (Dh, Dh)).T

        def wo_dot(r0, n):
            lhs = jnp.concatenate(lhs_o[r0 // Dh:(r0 + n) // Dh], axis=1)
            return _dot(lhs, wob[pl.ds(r0, n), :])

        row_d = lax.broadcasted_iota(jnp.int32, (R, D), 0)
        acc = jnp.where(row_d == 0, x + xn, 0.0)
        wait("wo", 0)
        for part in range(2):
            bump()
            acc = acc + wo_dot(part * (T0 // 2), T0 // 2)

        wait("wg")
        gt = _rnd(_dot(xn8, wgb[...]))
        gt = _rnd(gt * jax.nn.sigmoid(gt))
        up = None
        for i, (lo, hi) in enumerate(u_split):
            if i == len(u_split) - 1:
                wait("wd", 0)
            wait("wu%d" % i)
            w_rows = [wub[pl.ds(g * FR + lo, hi - lo), :] for g in range(GF)]
            t = _dot(xu[i], jnp.concatenate(w_rows, axis=0))
            up = t if up is None else up + t
        hh = (gt * _rnd(up)).astype(_BF16)
        y = _rnd(_dot(hh, wdb[...])) * r_sel
        acc = acc + jnp.where(row_d == 0, y, 0.0)

        for i, (r0, n, _) in enumerate(tail_mxu):
            wait("t%d" % i)
            acc = acc + wo_dot(r0, n)
        accs = [acc[:, c * _LANES:(c + 1) * _LANES] for c in range(NC)]
        for i, (r0, n, _) in enumerate(tail_vpu):
            cf = [coef_ref[pl.ds(r0 - v0 + t, _SUB), :] for t in range(0, n, _SUB)]
            wait("t%d" % (len(tail_mxu) + i))
            w = wob[pl.ds(r0, n), :].astype(_F32)
            for c in range(NC):
                prods = [w[t * _SUB:(t + 1) * _SUB, c * _LANES:(c + 1) * _LANES] * cf[t]
                         for t in range(n // _SUB)]
                accs[c] = accs[c] + _tree_sum(prods)
        assert issued[0] == len(stream)
        res = jnp.sum(jnp.concatenate(accs, axis=1), axis=0, keepdims=True)
        o_ref[...] = res.astype(o_ref.dtype)

    any_spec = pl.BlockSpec(memory_space=pl.ANY)
    out = pl.pallas_call(
        kernel,
        out_shape=jax.ShapeDtypeStruct((1, D), A_x.dtype),
        in_specs=[any_spec] * 9,
        out_specs=pl.BlockSpec(memory_space=pltpu.VMEM),
        scratch_shapes=[
            pltpu.VMEM((1, D), _BF16),
            pltpu.VMEM((NC, _LANES), _BF16),
            pltpu.VMEM((Hkv, W, Dh), _BF16),
            pltpu.VMEM((Hkv, W, Dh), _BF16),
            pltpu.VMEM((D, Hq * Dh), _BF16),
            pltpu.VMEM((Hq * Dh, D), _BF16),
            pltpu.VMEM((D, F), _BF16),
            pltpu.VMEM((D, F), _BF16),
            pltpu.VMEM((F, D), _BF16),
            pltpu.VMEM((Hq * Dh - v0, Dh), _F32),
        ],
        compiler_params=pltpu.CompilerParams(vmem_limit_bytes=64 * 1024 * 1024),
    )(A_x.reshape(1, D), B_w_r.reshape(NC, _LANES), A_k_cache, A_v_cache,
      A_wq, A_wo, B_w_gate, B_w_up, B_w_down)
    return out.reshape(B, Sq, D)
```

```python
import jax
import jax.numpy as jnp
from jax import lax
import jax.experimental.pallas as pl
import jax.experimental.pallas.tpu as pltpu

_F32 = jnp.float32
_BF16 = jnp.bfloat16
_LANES = 128
_SUB = 8


def _dot(a, b):
    return jnp.dot(a, b, preferred_element_type=_F32)


def _dot_nt(a, b):
    return lax.dot_general(a, b, (((1,), (1,)), ((), ())), preferred_element_type=_F32)


def _rnd(a):
    return a.astype(_BF16).astype(_F32)


def _tree_sum(xs):
    xs = list(xs)
    while len(xs) > 1:
        nxt = [xs[i] + xs[i + 1] for i in range(0, len(xs) - 1, 2)]
        if len(xs) % 2:
            nxt.append(xs[-1])
        xs = nxt
    return xs[0]


def _rects(t0, t1, c):
    out = []
    if t0 % c:
        e = min(t1, (t0 // c + 1) * c)
        out.append((pl.ds(t0 // c * _SUB, _SUB), pl.ds(t0 % c * _LANES, (e - t0) * _LANES)))
        t0 = e
    if t1 // c > t0 // c:
        out.append((pl.ds(t0 // c * _SUB, (t1 // c - t0 // c) * _SUB), pl.ds(0, c * _LANES)))
        t0 = t1 // c * c
    if t1 > t0:
        out.append((pl.ds(t0 // c * _SUB, _SUB), pl.ds(0, (t1 - t0) * _LANES)))
    return out


def _cut(lo, hi, phase, size):
    cuts = [lo] + [t for t in range(lo + 1, hi) if t % size == phase % size] + [hi]
    return list(zip(cuts[:-1], cuts[1:]))


def _round_robin(parts):
    return [p[i] for i in range(max(map(len, parts))) for p in parts if i < len(p)]


def _hop(items, regions):
    n = -(-len(items) // regions)
    return _round_robin([items[g * n:(g + 1) * n] for g in range(regions)])


@jax.jit
def pallas_parallel_sum__sliding_block_cached__moe_arch_mod__decode_kernel(
    A_x: jax.Array,
    A_k_cache: jax.Array,
    A_v_cache: jax.Array,
    A_wq: jax.Array,
    A_wo: jax.Array,
    B_x: jax.Array,
    B_w_r: jax.Array,
    B_w_gate: jax.Array,
    B_w_up: jax.Array,
    B_w_down: jax.Array,
):
    del B_x
    B, Sq, D = A_x.shape
    Hq, Dh = 32, 128
    Hkv, Sk = A_k_cache.shape[1], A_k_cache.shape[2]
    W = min(4096, max(256, Sk // 4))
    rep = Hq // Hkv
    F = B_w_gate.shape[1]
    assert (B, Sq, D, Hkv, W, F) == (1, 1, 512, 8, 4096, 1792)
    R = _SUB
    G = rep * Dh
    NC = D // _LANES

    BIG, SMALL = 16, 4
    PH_A, PH_B = 14, 15
    AHEAD = 140
    BUMP = 20
    LAST = 48
    GQ, GF = 8, 4
    NB = 8
    KB = W // NB
    FR = D // GF
    u_split = [(0, 96), (96, FR)]
    T0 = 3072
    tail_mxu = [(3072, 512, 32), (3584, 256, 16)]
    tail_vpu = [(3840, 128, 16), (3968, 64, 16), (4032, 32, 16), (4064, 32, 16)]
    v0 = tail_vpu[0][0]
    n_mxu_heads = v0 // Dh
    n_groups = 2 + 2 * NB + 1 + len(u_split) + len(tail_mxu) + len(tail_vpu) + 2

    def kernel(*refs):
        pl.run_scoped(lambda sems: body(*refs, sems),
                      pltpu.SemaphoreType.DMA((n_groups,)))

    def body(x_hbm, wr_hbm, k_hbm, v_hbm, wq_hbm, wo_hbm, wg_hbm, wu_hbm, wd_hbm,
             o_ref,
             xb, wrb, kb, vb, wqb, wob, wgb, wub, wdb, coef_ref, sems):
        groups = {}
        main, woven = [], []

        def group(name, *regions):
            groups[name] = (sems.at[len(groups)], regions)

        def piece(name, src, dst, t0, t1):
            return [(name, src.at[idx], dst.at[idx])
                    for idx in _rects(t0, t1, dst.shape[1] // _LANES)]

        def tiles(ref, rows=None):
            return (ref.shape[0] if rows is None else rows) // _SUB * (ref.shape[1] // _LANES)

        group("x", xb, wrb)
        group("q", wqb)
        for a, b in _hop(_cut(0, tiles(wqb), PH_A, BIG), GQ):
            main.append(piece("q", wq_hbm, wqb, a, b))
        kv_bounds = [0] + [b * KB // _SUB + PH_A for b in range(1, NB)] + [W // _SUB]
        for nm, src, dst in (("k", k_hbm, kb), ("v", v_hbm, vb)):
            for b in range(NB):
                lo, hi = kv_bounds[b], kv_bounds[b + 1]
                group("%s%d" % (nm, b), dst.at[:, pl.ds(lo * _SUB, (hi - lo) * _SUB)])
                for a, e in _cut(lo, hi, PH_A, BIG):
                    for h in range(Hkv):
                        main.append(piece("%s%d" % (nm, b), src.at[0, h, pl.ds(Sk - W, W)],
                                          dst.at[h], a, e))
        group("wg", wgb)
        for a, b in _hop(_cut(0, tiles(wgb), PH_B, BIG), GF):
            main.append(piece("wg", wg_hbm, wgb, a, b))
        u_parts, u_regions = ([], []), ([], [])
        for g in range(GF):
            lo, hi = tiles(wub, g * FR), tiles(wub, (g + 1) * FR)
            cuts = _cut(lo, hi, PH_B, BIG)
            first = [c for c in cuts if c[0] < tiles(wub, g * FR + u_split[0][1])]
            mid = first[-1][1]
            u_parts[0].append(first)
            u_parts[1].append(cuts[len(first):])
            u_regions[0].extend(wub.at[idx] for idx in _rects(lo, mid, F // _LANES))
            u_regions[1].extend(wub.at[idx] for idx in _rects(mid, hi, F // _LANES))
        for i in range(2):
            group("wu%d" % i, *u_regions[i])
            for a, b in _round_robin(u_parts[i]):
                main.append(piece("wu%d" % i, wu_hbm, wub, a, b))
        for i, (r0, n, rows) in enumerate(tail_mxu + tail_vpu):
            group("t%d" % i, wob.at[pl.ds(r0, n)])
            for r in range(r0, r0 + n, rows):
                main.append(piece("t%d" % i, wo_hbm, wob, tiles(wob, r), tiles(wob, r + rows)))
        group("wo", wob.at[pl.ds(0, T0)])
        for a, b in _hop(_cut(0, tiles(wob, T0), PH_A, SMALL), GF):
            woven.append(piece("wo", wo_hbm, wob, a, b))
        group("wd", wdb)
        for a, b in _hop(_cut(0, tiles(wdb), 0, SMALL), GF):
            woven.append(piece("wd", wd_hbm, wdb, a, b))
        assert len(groups) == n_groups

        stream = []
        span = len(main) - LAST
        n_w = 0
        for i, p in enumerate(main):
            stream.extend(c + (1,) for c in p)
            if i == 0:
                stream.append(("x", x_hbm, xb, 0))
                stream.append(("x", wr_hbm, wrb, 0))
            while n_w < len(woven) and n_w * span < (i + 1) * len(woven):
                stream.extend(c + (0,) for c in woven[n_w])
                n_w += 1
        assert n_w == len(woven)
        last = {c[0]: i for i, c in enumerate(stream)}
        issued = [0]

        def issue_to(n):
            for i in range(issued[0], min(n, len(stream))):
                name, src, dst, prio = stream[i]
                pltpu.make_async_copy(src, dst, groups[name][0]).start(priority=prio)
                issued[0] = i + 1

        def bump():
            issue_to(issued[0] + BUMP)

        def wait(name, ahead=AHEAD):
            issue_to(last[name] + 1 + ahead)
            sem, regions = groups[name]
            for reg in regions:
                pltpu.make_async_copy(reg, reg, sem).wait()

        wait("x")
        x = xb[...].astype(_F32)
        m = jnp.mean(x, axis=-1, keepdims=True)
        xc = x - m
        var = jnp.mean(xc * xc, axis=-1, keepdims=True)
        eps = _rnd(jnp.full((1, 1), 1e-5, _F32))
        den = _rnd(jnp.sqrt(_rnd(_rnd(var) + eps)))
        xn = _rnd(_rnd(x - _rnd(m)) / den)
        xn8f = jnp.broadcast_to(xn, (R, D))
        xn8 = xn8f.astype(_BF16)
        xu = [jnp.concatenate([xn8f[:, g * FR + lo:g * FR + hi] for g in range(GF)],
                              axis=1).astype(_BF16) for lo, hi in u_split]
        wr = wrb[...].astype(_F32)
        racc = xn[:, 0:_LANES] * wr[0:1, :]
        for j in range(1, NC):
            racc = racc + xn[:, j * _LANES:(j + 1) * _LANES] * wr[j:j + 1, :]
        r_sel = _rnd(jax.nn.sigmoid(_rnd(jnp.sum(racc, axis=-1, keepdims=True))))
        scale = _rnd(jnp.full((1, 1), Dh ** -0.5, _F32))
        row = lax.broadcasted_iota(jnp.int32, (R, Dh), 0)

        wait("q")
        qs = []
        half = Hkv // 2
        for part in range(2):
            if part:
                bump()
            q8 = _dot(xn8, wqb[:, pl.ds(part * half * G, half * G)])
            for h in range(half):
                qh = q8[:, h * G:h * G + Dh]
                for j in range(1, rep):
                    qh = jnp.where(row == j, q8[:, h * G + j * Dh:h * G + (j + 1) * Dh], qh)
                qs.append(qh.astype(_BF16))

        s = [[] for _ in range(Hkv)]
        for b in range(NB):
            wait("k%d" % b)
            for h in range(Hkv):
                s[h].append(_rnd(_rnd(_dot_nt(qs[h], kb[h, pl.ds(b * KB, KB), :])) * scale))
        bump()
        ps, ls = [], []
        for h in range(Hkv):
            sh = jnp.concatenate(s[h], axis=1)
            mx = jnp.max(sh, axis=-1, keepdims=True)
            p = jnp.exp(_rnd(sh - mx)).astype(_BF16)
            ps.append(p)
            ls.append(jnp.sum(p.astype(_F32), axis=-1, keepdims=True))
        pv = [None] * Hkv
        for b in range(NB):
            wait("v%d" % b)
            for h in range(Hkv):
                t = _dot(ps[h][:, b * KB:(b + 1) * KB], vb[h, pl.ds(b * KB, KB), :])
                pv[h] = t if pv[h] is None else pv[h] + t
        lhs_o = []
        for h in range(Hkv):
            oh = pv[h] / ls[h]
            for j in range(rep):
                if h * rep + j < n_mxu_heads:
                    lhs_o.append(jnp.where(row == j, oh, 0.0).astype(_BF16))
                else:
                    c0 = (h * rep + j) * Dh - v0
                    coef_ref[pl.ds(c0, Dh), :] = jnp.broadcast_to(_rnd(oh[j:j + 1, :]), (Dh, Dh)).T

        def wo_dot(r0, n):
            lhs = jnp.concatenate(lhs_o[r0 // Dh:(r0 + n) // Dh], axis=1)
            return _dot(lhs, wob[pl.ds(r0, n), :])

        row_d = lax.broadcasted_iota(jnp.int32, (R, D), 0)
        acc = jnp.where(row_d == 0, x + xn, 0.0)
        wait("wo", 0)
        for part in range(2):
            bump()
            acc = acc + wo_dot(part * (T0 // 2), T0 // 2)

        wait("wg")
        gt = _rnd(_dot(xn8, wgb[...]))
        gt = _rnd(gt * jax.nn.sigmoid(gt))
        up = None
        for i, (lo, hi) in enumerate(u_split):
            if i == len(u_split) - 1:
                wait("wd", 0)
            wait("wu%d" % i)
            w_rows = [wub[pl.ds(g * FR + lo, hi - lo), :] for g in range(GF)]
            t = _dot(xu[i], jnp.concatenate(w_rows, axis=0))
            up = t if up is None else up + t
        hh = (gt * _rnd(up)).astype(_BF16)
        y = _rnd(_dot(hh, wdb[...])) * r_sel
        acc = acc + jnp.where(row_d == 0, y, 0.0)

        for i, (r0, n, _) in enumerate(tail_mxu):
            wait("t%d" % i)
            acc = acc + wo_dot(r0, n)
        accs = [acc[:, c * _LANES:(c + 1) * _LANES] for c in range(NC)]
        for i, (r0, n, _) in enumerate(tail_vpu):
            cf = [coef_ref[pl.ds(r0 - v0 + t, _SUB), :] for t in range(0, n, _SUB)]
            wait("t%d" % (len(tail_mxu) + i))
            w = wob[pl.ds(r0, n), :].astype(_F32)
            for c in range(NC):
                prods = [w[t * _SUB:(t + 1) * _SUB, c * _LANES:(c + 1) * _LANES] * cf[t]
                         for t in range(n // _SUB)]
                accs[c] = accs[c] + _tree_sum(prods)
        assert issued[0] == len(stream)
        res = jnp.sum(jnp.concatenate(accs, axis=1), axis=0, keepdims=True)
        o_ref[...] = res.astype(o_ref.dtype)

    any_spec = pl.BlockSpec(memory_space=pl.ANY)
    out = pl.pallas_call(
        kernel,
        out_shape=jax.ShapeDtypeStruct((1, D), A_x.dtype),
        in_specs=[any_spec] * 9,
        out_specs=pl.BlockSpec(memory_space=pltpu.VMEM),
        scratch_shapes=[
            pltpu.VMEM((1, D), _BF16),
            pltpu.VMEM((NC, _LANES), _BF16),
            pltpu.VMEM((Hkv, W, Dh), _BF16),
            pltpu.VMEM((Hkv, W, Dh), _BF16),
            pltpu.VMEM((D, Hq * Dh), _BF16),
            pltpu.VMEM((Hq * Dh, D), _BF16),
            pltpu.VMEM((D, F), _BF16),
            pltpu.VMEM((D, F), _BF16),
            pltpu.VMEM((F, D), _BF16),
            pltpu.VMEM((Hq * Dh - v0, Dh), _F32),
        ],
        compiler_params=pltpu.CompilerParams(vmem_limit_bytes=64 * 1024 * 1024),
    )(A_x.reshape(1, D), B_w_r.reshape(NC, _LANES), A_k_cache, A_v_cache,
      A_wq, A_wo, B_w_gate, B_w_up, B_w_down)
    return out.reshape(B, Sq, D)
```

```python
import jax
import jax.numpy as jnp
from jax import lax
import jax.experimental.pallas as pl
import jax.experimental.pallas.tpu as pltpu

_F32 = jnp.float32
_BF16 = jnp.bfloat16
_LANES = 128
_SUB = 8


def _dot(a, b):
    return jnp.dot(a, b, preferred_element_type=_F32)


def _dot_nt(a, b):
    return lax.dot_general(a, b, (((1,), (1,)), ((), ())), preferred_element_type=_F32)


def _rnd(a):
    return a.astype(_BF16).astype(_F32)


def _tree_sum(xs):
    xs = list(xs)
    while len(xs) > 1:
        nxt = [xs[i] + xs[i + 1] for i in range(0, len(xs) - 1, 2)]
        if len(xs) % 2:
            nxt.append(xs[-1])
        xs = nxt
    return xs[0]


def _rects(t0, t1, c):
    out = []
    if t0 % c:
        e = min(t1, (t0 // c + 1) * c)
        out.append((pl.ds(t0 // c * _SUB, _SUB), pl.ds(t0 % c * _LANES, (e - t0) * _LANES)))
        t0 = e
    if t1 // c > t0 // c:
        out.append((pl.ds(t0 // c * _SUB, (t1 // c - t0 // c) * _SUB), pl.ds(0, c * _LANES)))
        t0 = t1 // c * c
    if t1 > t0:
        out.append((pl.ds(t0 // c * _SUB, _SUB), pl.ds(0, (t1 - t0) * _LANES)))
    return out


def _cut(lo, hi, phase, size):
    cuts = [lo] + [t for t in range(lo + 1, hi) if t % size == phase % size] + [hi]
    return list(zip(cuts[:-1], cuts[1:]))


def _round_robin(parts):
    return [p[i] for i in range(max(map(len, parts))) for p in parts if i < len(p)]


def _hop(items, regions):
    n = -(-len(items) // regions)
    return _round_robin([items[g * n:(g + 1) * n] for g in range(regions)])


@jax.jit
def pallas_parallel_sum__sliding_block_cached__moe_arch_mod__decode_kernel(
    A_x: jax.Array,
    A_k_cache: jax.Array,
    A_v_cache: jax.Array,
    A_wq: jax.Array,
    A_wo: jax.Array,
    B_x: jax.Array,
    B_w_r: jax.Array,
    B_w_gate: jax.Array,
    B_w_up: jax.Array,
    B_w_down: jax.Array,
):
    del B_x
    B, Sq, D = A_x.shape
    Hq, Dh = 32, 128
    Hkv, Sk = A_k_cache.shape[1], A_k_cache.shape[2]
    W = min(4096, max(256, Sk // 4))
    rep = Hq // Hkv
    F = B_w_gate.shape[1]
    assert (B, Sq, D, Hkv, W, F) == (1, 1, 512, 8, 4096, 1792)
    R = _SUB
    G = rep * Dh
    NC = D // _LANES

    BIG, SMALL = 16, 4
    PH_A, PH_B = 14, 15
    AHEAD = 140
    BUMP = 20
    LAST = 48
    GQ, GF = 8, 4
    NB = 8
    KB = W // NB
    FR = D // GF
    u_split = [(0, 96), (96, FR)]
    T0 = 3072
    tail_mxu = [(3072, 512, 32), (3584, 256, 16)]
    tail_vpu = [(3840, 128, 16), (3968, 64, 16), (4032, 32, 16), (4064, 32, 16)]
    v0 = tail_vpu[0][0]
    n_mxu_heads = v0 // Dh
    n_groups = 2 + 2 * NB + 1 + len(u_split) + len(tail_mxu) + len(tail_vpu) + 2

    def kernel(*refs):
        pl.run_scoped(lambda sems: body(*refs, sems),
                      pltpu.SemaphoreType.DMA((n_groups,)))

    def body(x_hbm, wr_hbm, k_hbm, v_hbm, wq_hbm, wo_hbm, wg_hbm, wu_hbm, wd_hbm,
             o_ref,
             xb, wrb, kb, vb, wqb, wob, wgb, wub, wdb, coef_ref, sems):
        groups = {}
        main, woven = [], []

        def group(name, region=None):
            groups[name] = (sems.at[len(groups)], region)

        def piece(name, src, dst, t0, t1):
            return [(name, src.at[idx], dst.at[idx])
                    for idx in _rects(t0, t1, dst.shape[1] // _LANES)]

        def tiles(ref, rows=None):
            return (ref.shape[0] if rows is None else rows) // _SUB * (ref.shape[1] // _LANES)

        group("x")
        group("q", wqb)
        for a, b in _hop(_cut(0, tiles(wqb), PH_A, BIG), GQ):
            main.append(piece("q", wq_hbm, wqb, a, b))
        kv_bounds = [0] + [b * KB // _SUB + PH_A for b in range(1, NB)] + [W // _SUB]
        for nm, src, dst in (("k", k_hbm, kb), ("v", v_hbm, vb)):
            for b in range(NB):
                lo, hi = kv_bounds[b], kv_bounds[b + 1]
                group("%s%d" % (nm, b), dst.at[:, pl.ds(lo * _SUB, (hi - lo) * _SUB)])
                for a, e in _cut(lo, hi, PH_A, BIG):
                    for h in range(Hkv):
                        main.append(piece("%s%d" % (nm, b), src.at[0, h, pl.ds(Sk - W, W)],
                                          dst.at[h], a, e))
        group("wg", wgb)
        for a, b in _hop(_cut(0, tiles(wgb), PH_B, BIG), GF):
            main.append(piece("wg", wg_hbm, wgb, a, b))
        u_parts = ([], [])
        for g in range(GF):
            cuts = _cut(tiles(wub, g * FR), tiles(wub, (g + 1) * FR), PH_B, BIG)
            first = [c for c in cuts if c[0] < tiles(wub, g * FR + u_split[0][1])]
            u_parts[0].append(first)
            u_parts[1].append(cuts[len(first):])
        for i in range(2):
            group("wu%d" % i)
            for a, b in _round_robin(u_parts[i]):
                main.append(piece("wu%d" % i, wu_hbm, wub, a, b))
        for i, (r0, n, rows) in enumerate(tail_mxu + tail_vpu):
            group("t%d" % i, wob.at[pl.ds(r0, n)])
            for r in range(r0, r0 + n, rows):
                main.append(piece("t%d" % i, wo_hbm, wob, tiles(wob, r), tiles(wob, r + rows)))
        group("wo", wob.at[pl.ds(0, T0)])
        for a, b in _hop(_cut(0, tiles(wob, T0), PH_A, SMALL), GF):
            woven.append(piece("wo", wo_hbm, wob, a, b))
        group("wd", wdb)
        for a, b in _hop(_cut(0, tiles(wdb), 0, SMALL), GF):
            woven.append(piece("wd", wd_hbm, wdb, a, b))
        assert len(groups) == n_groups

        stream = []
        span = len(main) - LAST
        n_w = 0
        for i, p in enumerate(main):
            stream.extend(c + (1,) for c in p)
            if i == 0:
                stream.append(("x", x_hbm, xb, 0))
                stream.append(("x", wr_hbm, wrb, 0))
            while n_w < len(woven) and n_w * span < (i + 1) * len(woven):
                stream.extend(c + (0,) for c in woven[n_w])
                n_w += 1
        assert n_w == len(woven)
        last = {c[0]: i for i, c in enumerate(stream)}
        issued = [0]

        def issue_to(n):
            for i in range(issued[0], min(n, len(stream))):
                name, src, dst, prio = stream[i]
                pltpu.make_async_copy(src, dst, groups[name][0]).start(priority=prio)
                issued[0] = i + 1

        def bump():
            issue_to(issued[0] + BUMP)

        def wait(name, ahead=AHEAD):
            issue_to(last[name] + 1 + ahead)
            sem, region = groups[name]
            if region is not None:
                pltpu.make_async_copy(region, region, sem).wait()
            else:
                for g_name, src, dst, _ in stream:
                    if g_name == name:
                        pltpu.make_async_copy(src, dst, sem).wait()

        wait("x")
        x = xb[...].astype(_F32)
        m = jnp.mean(x, axis=-1, keepdims=True)
        xc = x - m
        var = jnp.mean(xc * xc, axis=-1, keepdims=True)
        eps = _rnd(jnp.full((1, 1), 1e-5, _F32))
        den = _rnd(jnp.sqrt(_rnd(_rnd(var) + eps)))
        xn = _rnd(_rnd(x - _rnd(m)) / den)
        xn8f = jnp.broadcast_to(xn, (R, D))
        xn8 = xn8f.astype(_BF16)
        xu = [jnp.concatenate([xn8f[:, g * FR + lo:g * FR + hi] for g in range(GF)],
                              axis=1).astype(_BF16) for lo, hi in u_split]
        wr = wrb[...].astype(_F32)
        racc = xn[:, 0:_LANES] * wr[0:1, :]
        for j in range(1, NC):
            racc = racc + xn[:, j * _LANES:(j + 1) * _LANES] * wr[j:j + 1, :]
        r_sel = _rnd(jax.nn.sigmoid(_rnd(jnp.sum(racc, axis=-1, keepdims=True))))
        scale = _rnd(jnp.full((1, 1), Dh ** -0.5, _F32))
        row = lax.broadcasted_iota(jnp.int32, (R, Dh), 0)

        wait("q")
        qs = []
        half = Hkv // 2
        for part in range(2):
            if part:
                bump()
            q8 = _dot(xn8, wqb[:, pl.ds(part * half * G, half * G)])
            for h in range(half):
                qh = q8[:, h * G:h * G + Dh]
                for j in range(1, rep):
                    qh = jnp.where(row == j, q8[:, h * G + j * Dh:h * G + (j + 1) * Dh], qh)
                qs.append(qh.astype(_BF16))

        s = [[] for _ in range(Hkv)]
        for b in range(NB):
            wait("k%d" % b)
            for h in range(Hkv):
                s[h].append(_rnd(_rnd(_dot_nt(qs[h], kb[h, pl.ds(b * KB, KB), :])) * scale))
        bump()
        ps, ls = [], []
        for h in range(Hkv):
            sh = jnp.concatenate(s[h], axis=1)
            mx = jnp.max(sh, axis=-1, keepdims=True)
            p = jnp.exp(_rnd(sh - mx)).astype(_BF16)
            ps.append(p)
            ls.append(jnp.sum(p.astype(_F32), axis=-1, keepdims=True))
        pv = [None] * Hkv
        for b in range(NB):
            wait("v%d" % b)
            for h in range(Hkv):
                t = _dot(ps[h][:, b * KB:(b + 1) * KB], vb[h, pl.ds(b * KB, KB), :])
                pv[h] = t if pv[h] is None else pv[h] + t
        lhs_o = []
        for h in range(Hkv):
            oh = pv[h] / ls[h]
            for j in range(rep):
                if h * rep + j < n_mxu_heads:
                    lhs_o.append(jnp.where(row == j, oh, 0.0).astype(_BF16))
                else:
                    c0 = (h * rep + j) * Dh - v0
                    coef_ref[pl.ds(c0, Dh), :] = jnp.broadcast_to(_rnd(oh[j:j + 1, :]), (Dh, Dh)).T

        def wo_dot(r0, n):
            lhs = jnp.concatenate(lhs_o[r0 // Dh:(r0 + n) // Dh], axis=1)
            return _dot(lhs, wob[pl.ds(r0, n), :])

        row_d = lax.broadcasted_iota(jnp.int32, (R, D), 0)
        acc = jnp.where(row_d == 0, x + xn, 0.0)
        wait("wo", 0)
        for part in range(2):
            bump()
            acc = acc + wo_dot(part * (T0 // 2), T0 // 2)

        wait("wg")
        gt = _rnd(_dot(xn8, wgb[...]))
        gt = _rnd(gt * jax.nn.sigmoid(gt))
        up = None
        for i, (lo, hi) in enumerate(u_split):
            if i == len(u_split) - 1:
                wait("wd", 0)
            wait("wu%d" % i)
            w_rows = [wub[pl.ds(g * FR + lo, hi - lo), :] for g in range(GF)]
            t = _dot(xu[i], jnp.concatenate(w_rows, axis=0))
            up = t if up is None else up + t
        hh = (gt * _rnd(up)).astype(_BF16)
        y = _rnd(_dot(hh, wdb[...])) * r_sel
        acc = acc + jnp.where(row_d == 0, y, 0.0)

        for i, (r0, n, _) in enumerate(tail_mxu):
            wait("t%d" % i)
            acc = acc + wo_dot(r0, n)
        accs = [acc[:, c * _LANES:(c + 1) * _LANES] for c in range(NC)]
        for i, (r0, n, _) in enumerate(tail_vpu):
            cf = [coef_ref[pl.ds(r0 - v0 + t, _SUB), :] for t in range(0, n, _SUB)]
            wait("t%d" % (len(tail_mxu) + i))
            w = wob[pl.ds(r0, n), :].astype(_F32)
            for c in range(NC):
                prods = [w[t * _SUB:(t + 1) * _SUB, c * _LANES:(c + 1) * _LANES] * cf[t]
                         for t in range(n // _SUB)]
                accs[c] = accs[c] + _tree_sum(prods)
        assert issued[0] == len(stream)
        res = jnp.sum(jnp.concatenate(accs, axis=1), axis=0, keepdims=True)
        o_ref[...] = res.astype(o_ref.dtype)

    any_spec = pl.BlockSpec(memory_space=pl.ANY)
    out = pl.pallas_call(
        kernel,
        out_shape=jax.ShapeDtypeStruct((1, D), A_x.dtype),
        in_specs=[any_spec] * 9,
        out_specs=pl.BlockSpec(memory_space=pltpu.VMEM),
        scratch_shapes=[
            pltpu.VMEM((1, D), _BF16),
            pltpu.VMEM((NC, _LANES), _BF16),
            pltpu.VMEM((Hkv, W, Dh), _BF16),
            pltpu.VMEM((Hkv, W, Dh), _BF16),
            pltpu.VMEM((D, Hq * Dh), _BF16),
            pltpu.VMEM((Hq * Dh, D), _BF16),
            pltpu.VMEM((D, F), _BF16),
            pltpu.VMEM((D, F), _BF16),
            pltpu.VMEM((F, D), _BF16),
            pltpu.VMEM((Hq * Dh - v0, Dh), _F32),
        ],
        compiler_params=pltpu.CompilerParams(vmem_limit_bytes=64 * 1024 * 1024),
    )(A_x.reshape(1, D), B_w_r.reshape(NC, _LANES), A_k_cache, A_v_cache,
      A_wq, A_wo, B_w_gate, B_w_up, B_w_down)
    return out.reshape(B, Sq, D)
```

```python
import jax
import jax.numpy as jnp
from jax import lax
import jax.experimental.pallas as pl
import jax.experimental.pallas.tpu as pltpu

_F32 = jnp.float32
_BF16 = jnp.bfloat16
_LANES = 128
_SUB = 8


def _dot(a, b):
    return jnp.dot(a, b, preferred_element_type=_F32)


def _dot_nt(a, b):
    return lax.dot_general(a, b, (((1,), (1,)), ((), ())), preferred_element_type=_F32)


def _rnd(a):
    return a.astype(_BF16).astype(_F32)


def _tree_sum(xs):
    xs = list(xs)
    while len(xs) > 1:
        nxt = [xs[i] + xs[i + 1] for i in range(0, len(xs) - 1, 2)]
        if len(xs) % 2:
            nxt.append(xs[-1])
        xs = nxt
    return xs[0]


def _rects(t0, t1, c):
    out = []
    if t0 % c:
        e = min(t1, (t0 // c + 1) * c)
        out.append((pl.ds(t0 // c * _SUB, _SUB), pl.ds(t0 % c * _LANES, (e - t0) * _LANES)))
        t0 = e
    if t1 // c > t0 // c:
        out.append((pl.ds(t0 // c * _SUB, (t1 // c - t0 // c) * _SUB), pl.ds(0, c * _LANES)))
        t0 = t1 // c * c
    if t1 > t0:
        out.append((pl.ds(t0 // c * _SUB, _SUB), pl.ds(0, (t1 - t0) * _LANES)))
    return out


def _cut(lo, hi, phase, size):
    cuts = [lo] + [t for t in range(lo + 1, hi) if t % size == phase % size] + [hi]
    return list(zip(cuts[:-1], cuts[1:]))


def _hop(items, regions):
    n = -(-len(items) // regions)
    parts = [items[g * n:(g + 1) * n] for g in range(regions)]
    return [p[i] for i in range(n) for p in parts if i < len(p)]


def _merge(base, extra, end):
    keyed = [((i + 0.5) / len(base), 0, i, p) for i, p in enumerate(base)]
    keyed += [(end * (i + 0.5) / len(extra), 1, i, p) for i, p in enumerate(extra)]
    return [k[3] for k in sorted(keyed, key=lambda k: k[:3])]


@jax.jit
def pallas_parallel_sum__sliding_block_cached__moe_arch_mod__decode_kernel(
    A_x: jax.Array,
    A_k_cache: jax.Array,
    A_v_cache: jax.Array,
    A_wq: jax.Array,
    A_wo: jax.Array,
    B_x: jax.Array,
    B_w_r: jax.Array,
    B_w_gate: jax.Array,
    B_w_up: jax.Array,
    B_w_down: jax.Array,
):
    del B_x
    B, Sq, D = A_x.shape
    Hq, Dh = 32, 128
    Hkv, Sk = A_k_cache.shape[1], A_k_cache.shape[2]
    W = min(4096, max(256, Sk // 4))
    rep = Hq // Hkv
    F = B_w_gate.shape[1]
    assert (B, Sq, D, Hkv, W, F) == (1, 1, 512, 8, 4096, 1792)
    R = _SUB
    G = rep * Dh
    NC = D // _LANES
    half = Hkv // 2

    BIG, SMALL = 16, 4
    PH_A, PH_B = 14, 15
    AHEAD = 140
    BUMP = 20
    LAST = 48
    GQ, GF = 8, 4
    NB = 8
    KB = W // NB
    FFN_AT = 5
    WD_AT = 100
    T0 = 3072
    tail_mxu = [(3072, 512, 32), (3584, 256, 16)]
    tail_vpu = [(3840, 128, 16), (3968, 64, 16), (4032, 32, 16), (4064, 16, 16), (4080, 16, 16)]
    v0 = tail_vpu[0][0]
    n_mxu_heads = v0 // Dh
    n_groups = 3 + 2 * NB + 1 + 2 + len(tail_mxu) + len(tail_vpu) + 2

    def kernel(*refs):
        pl.run_scoped(lambda sems: body(*refs, sems),
                      pltpu.SemaphoreType.DMA((n_groups,)))

    def body(x_hbm, wr_hbm, k_hbm, v_hbm, wq_hbm, wo_hbm, wg_hbm, wu_hbm, wd_hbm,
             o_ref,
             xb, wrb, kb, vb, wqb, wob, wgb, wub, wdb, coef_ref, sems):
        groups = {}

        def group(name, region):
            groups[name] = (sems.at[len(groups)], region)

        def piece(name, src, dst, t0, t1):
            return [(name, src.at[idx], dst.at[idx])
                    for idx in _rects(t0, t1, dst.shape[1] // _LANES)]

        def tiles(ref, rows=None):
            return (ref.shape[0] if rows is None else rows) // _SUB * (ref.shape[1] // _LANES)

        def hopping(name, src, dst, rows, phase, size, regions):
            group(name, dst.at[pl.ds(0, rows)])
            return [piece(name, src, dst, a, b)
                    for big in _hop(_cut(0, tiles(dst, rows), phase, BIG), regions)
                    for a, b in _cut(*big, phase, size)]

        group("x", xb)
        group("wr", wrb)
        main = hopping("q", wq_hbm, wqb, D, PH_A, BIG, GQ)
        kv_bounds = [0] + [b * KB // _SUB + PH_A for b in range(1, NB)] + [W // _SUB]
        kv = {"k": [], "v": []}
        for nm, src, dst in (("k", k_hbm, kb), ("v", v_hbm, vb)):
            for b in range(NB):
                lo, hi = kv_bounds[b], kv_bounds[b + 1]
                split = nm == "v" and b == NB - 1
                for part, (h0, h1) in enumerate([(0, half), (half, Hkv)] if split else [(0, Hkv)]):
                    name = "%s%d" % (nm, b + part)
                    group(name, dst.at[pl.ds(h0, h1 - h0), pl.ds(lo * _SUB, (hi - lo) * _SUB)])
                    for a, e in _cut(lo, hi, PH_A, BIG):
                        for h in range(h0, h1):
                            kv[nm].append(piece(name, src.at[0, h, pl.ds(Sk - W, W)],
                                                dst.at[h], a, e))
        main += _merge(kv["k"], hopping("wg", wg_hbm, wgb, D, PH_B, BIG, GF), 0.95)
        main += _merge(kv["v"], hopping("wu", wu_hbm, wub, D, PH_B, BIG, GF), 0.72)
        for i, (r0, n, rows) in enumerate(tail_mxu + tail_vpu):
            group("t%d" % i, wob.at[pl.ds(r0, n)])
            for r in range(r0, r0 + n, rows):
                main.append(piece("t%d" % i, wo_hbm, wob, tiles(wob, r), tiles(wob, r + rows)))
        woven = hopping("wo", wo_hbm, wob, T0, PH_A, SMALL, GF)
        woven[WD_AT:WD_AT] = hopping("wd", wd_hbm, wdb, F, 0, SMALL, GF)
        assert len(groups) == n_groups

        stream = []
        span = len(main) - LAST
        n_w = 0
        for i, p in enumerate(main):
            stream.extend(c + (1,) for c in p)
            if i == 0:
                stream.append(("x", x_hbm, xb, 0))
                stream.append(("wr", wr_hbm, wrb, 0))
            while n_w < len(woven) and n_w * span < (i + 1) * len(woven):
                stream.extend(c + (0,) for c in woven[n_w])
                n_w += 1
        assert n_w == len(woven)
        last = {c[0]: i for i, c in enumerate(stream)}
        issued = [0]

        def issue_to(n):
            for i in range(issued[0], min(n, len(stream))):
                name, src, dst, prio = stream[i]
                pltpu.make_async_copy(src, dst, groups[name][0]).start(priority=prio)
                issued[0] = i + 1

        def bump():
            issue_to(issued[0] + BUMP)

        def wait(name, ahead=AHEAD):
            issue_to(last[name] + 1 + ahead)
            sem, region = groups[name]
            pltpu.make_async_copy(region, region, sem).wait()

        wait("x")
        wait("wr")
        x = xb[...].astype(_F32)
        m = jnp.mean(x, axis=-1, keepdims=True)
        xc = x - m
        var = jnp.mean(xc * xc, axis=-1, keepdims=True)
        eps = _rnd(jnp.full((1, 1), 1e-5, _F32))
        den = _rnd(jnp.sqrt(_rnd(_rnd(var) + eps)))
        xn = _rnd(_rnd(x - _rnd(m)) / den)
        xn8 = jnp.broadcast_to(xn, (R, D)).astype(_BF16)
        wr = wrb[...].astype(_F32)
        racc = xn[:, 0:_LANES] * wr[0:1, :]
        for j in range(1, NC):
            racc = racc + xn[:, j * _LANES:(j + 1) * _LANES] * wr[j:j + 1, :]
        r_sel = _rnd(jax.nn.sigmoid(_rnd(jnp.sum(racc, axis=-1, keepdims=True))))
        scale = _rnd(jnp.full((1, 1), Dh ** -0.5, _F32))
        row = lax.broadcasted_iota(jnp.int32, (R, Dh), 0)
        row_d = lax.broadcasted_iota(jnp.int32, (R, D), 0)

        wait("q")
        qs = []
        for part in range(2):
            if part:
                bump()
            q8 = _dot(xn8, wqb[:, pl.ds(part * half * G, half * G)])
            for h in range(half):
                qh = q8[:, h * G:h * G + Dh]
                for j in range(1, rep):
                    qh = jnp.where(row == j, q8[:, h * G + j * Dh:h * G + (j + 1) * Dh], qh)
                qs.append(qh.astype(_BF16))

        s = [[] for _ in range(Hkv)]
        for b in range(NB):
            wait("k%d" % b)
            for h in range(Hkv):
                s[h].append(_rnd(_rnd(_dot_nt(qs[h], kb[h, pl.ds(b * KB, KB), :])) * scale))
        bump()
        ps, ls = [], []
        for h in range(Hkv):
            sh = jnp.concatenate(s[h], axis=1)
            mx = jnp.max(sh, axis=-1, keepdims=True)
            p = jnp.exp(_rnd(sh - mx)).astype(_BF16)
            ps.append(p)
            ls.append(jnp.sum(p.astype(_F32), axis=-1, keepdims=True))

        pv = [None] * Hkv

        def pv_block(b, heads):
            for h in heads:
                t = _dot(ps[h][:, b * KB:(b + 1) * KB], vb[h, pl.ds(b * KB, KB), :])
                pv[h] = t if pv[h] is None else pv[h] + t

        for b in range(NB - 1):
            wait("v%d" % b)
            pv_block(b, range(Hkv))
            if b == 0:
                wait("wg", 0)
                bump()
                gt = _rnd(_dot(xn8, wgb[...]))
                gt = _rnd(gt * jax.nn.sigmoid(gt))
            if b == FFN_AT:
                wait("wu", 0)
                wait("wd", 0)
                bump()
                hh = (gt * _rnd(_dot(xn8, wub[...]))).astype(_BF16)
                bump()
                y = _rnd(_dot(hh, wdb[...])) * r_sel
                acc = jnp.where(row_d == 0, (x + xn) + y, 0.0)

        lhs_o = []

        def wo_dot(r0, n):
            lhs = jnp.concatenate(lhs_o[r0 // Dh:(r0 + n) // Dh], axis=1)
            return _dot(lhs, wob[pl.ds(r0, n), :])

        wait("wo", 0)
        for part in range(2):
            heads = range(part * half, (part + 1) * half)
            wait("v%d" % (NB - 1 + part))
            pv_block(NB - 1, heads)
            for h in heads:
                oh = pv[h] / ls[h]
                for j in range(rep):
                    if h * rep + j < n_mxu_heads:
                        lhs_o.append(jnp.where(row == j, oh, 0.0).astype(_BF16))
                    else:
                        c0 = (h * rep + j) * Dh - v0
                        coef_ref[pl.ds(c0, Dh), :] = jnp.broadcast_to(
                            _rnd(oh[j:j + 1, :]), (Dh, Dh)).T
            r0 = part * half * G
            acc = acc + wo_dot(r0, min(T0, r0 + half * G) - r0)
        for i, (r0, n, _) in enumerate(tail_mxu):
            wait("t%d" % i)
            acc = acc + wo_dot(r0, n)
        accs = [acc[:, c * _LANES:(c + 1) * _LANES] for c in range(NC)]
        for i, (r0, n, _) in enumerate(tail_vpu):
            cf = [coef_ref[pl.ds(r0 - v0 + t, _SUB), :] for t in range(0, n, _SUB)]
            wait("t%d" % (len(tail_mxu) + i))
            w = wob[pl.ds(r0, n), :].astype(_F32)
            for c in range(NC):
                prods = [w[t * _SUB:(t + 1) * _SUB, c * _LANES:(c + 1) * _LANES] * cf[t]
                         for t in range(n // _SUB)]
                accs[c] = accs[c] + _tree_sum(prods)
        assert issued[0] == len(stream)
        res = jnp.sum(jnp.concatenate(accs, axis=1), axis=0, keepdims=True)
        o_ref[...] = res.astype(o_ref.dtype)

    any_spec = pl.BlockSpec(memory_space=pl.ANY)
    out = pl.pallas_call(
        kernel,
        out_shape=jax.ShapeDtypeStruct((1, D), A_x.dtype),
        in_specs=[any_spec] * 9,
        out_specs=pl.BlockSpec(memory_space=pltpu.VMEM),
        scratch_shapes=[
            pltpu.VMEM((1, D), _BF16),
            pltpu.VMEM((NC, _LANES), _BF16),
            pltpu.VMEM((Hkv, W, Dh), _BF16),
            pltpu.VMEM((Hkv, W, Dh), _BF16),
            pltpu.VMEM((D, Hq * Dh), _BF16),
            pltpu.VMEM((Hq * Dh, D), _BF16),
            pltpu.VMEM((D, F), _BF16),
            pltpu.VMEM((D, F), _BF16),
            pltpu.VMEM((F, D), _BF16),
            pltpu.VMEM((Hq * Dh - v0, Dh), _F32),
        ],
        compiler_params=pltpu.CompilerParams(vmem_limit_bytes=64 * 1024 * 1024),
    )(A_x.reshape(1, D), B_w_r.reshape(NC, _LANES), A_k_cache, A_v_cache,
      A_wq, A_wo, B_w_gate, B_w_up, B_w_down)
    return out.reshape(B, Sq, D)
```
